```python
import os as _os
_os.environ.setdefault("JAX_PLATFORMS", "cpu")
import jax
import jax.numpy as jnp

def _softmax(x, axis=-1):
    return jax.nn.softmax(x, axis=axis)
def _gelu(x):
    return jax.nn.gelu(x, approximate=True)
def _silu(x):
    return jax.nn.silu(x)
def _sigmoid(x):
    return jax.nn.sigmoid(x)
def _layernorm(x, axis=-1, eps=1e-5):
    m = jnp.mean(x, axis=axis, keepdims=True)
    v = jnp.var(x, axis=axis, keepdims=True)
    return (x - m) / jnp.sqrt(v + eps)
def _scatter_add(tgt, idx, src, axis=0):
    return tgt.at[idx].add(src)
def _segment_sum(src, seg, n):
    return jax.ops.segment_sum(src, seg, n)
class _Rng:
    def __init__(self, key):
        self._k = key
    def _next(self):
        self._k, sub = jax.random.split(self._k)
        return sub
    def normal(self, shape):
        return jax.random.normal(self._next(), shape, dtype=jnp.bfloat16)
    def randint(self, lo, hi, shape):
        return jax.random.randint(self._next(), shape, lo, hi, dtype=jnp.int32)
    def uniform(self, shape, lo=0.0, hi=1.0):
        return jax.random.uniform(self._next(), shape, jnp.bfloat16, lo, hi)
    def permutation(self, n):
        return jax.random.permutation(self._next(), n)


kernel_name = 'sequential_preLN__softmax_full_mha__dense_activation_gelu__prompt'

def setup_inputs():
    _rng = _Rng(jax.random.key(int.from_bytes(__import__("os").urandom(4), "little")))
    _w = (lambda a: (lambda t: t.astype(jnp.bfloat16) if jnp.issubdtype(t.dtype, jnp.floating) else t)(jnp.asarray(a)))
    def _A_setup():
        B, S, D = 1, 2048, 512
        return {
            "x": _w((lambda *s: _rng.normal(s) * 0.05)(B, S, D)),
            "wqkv": _w((lambda *s: _rng.normal(s) * 0.05)(D, 3 * D)),
            "wo": _w((lambda *s: _rng.normal(s) * 0.05)(D, D)),
        }
    _A_in = _A_setup()

    def _B_setup():
        B, S, D, F = 1, 2048, 512, 1792
        return {
            "x": _w((lambda *s: _rng.normal(s) * 0.05)(B, S, D)),
            "w1": _w((lambda *s: _rng.normal(s) * 0.4)(D, F) * (D ** -0.5)),
            "b1": _w((lambda *s: _rng.normal(s) * 0.4)(F) * 0.01),
            "w2": _w((lambda *s: _rng.normal(s) * 0.4)(F, D) * (F ** -0.5)),
            "b2": _w((lambda *s: _rng.normal(s) * 0.05)(D) * 0.01),
        }
    _B_in = _B_setup()

    return {
        "A_x": _A_in["x"],
        "A_wqkv": _A_in["wqkv"],
        "A_wo": _A_in["wo"],
        "B_x": _B_in["x"],
        "B_w1": _B_in["w1"],
        "B_b1": _B_in["b1"],
        "B_w2": _B_in["w2"],
        "B_b2": _B_in["b2"],
    }

def reference(A_x, A_wqkv, A_wo, B_x, B_w1, B_b1, B_w2, B_b2):
    def _A_ref(x, wqkv, wo):
        B, S, D = x.shape
        H = 32; Dh = D // H
        qkv = (lambda x, *d: x.transpose(*d))((x @ wqkv).reshape(B, S, 3, H, Dh), 2, 0, 3, 1, 4)
        q, k, v = qkv[0], qkv[1], qkv[2]
        scale = Dh ** -0.5
        scores = jnp.einsum("bhqd,bhkd->bhqk", q, k) * scale
        p = _softmax(scores, axis=-1)
        o = jnp.einsum("bhqk,bhkd->bhqd", p, v)
        return (lambda x, *d: x.transpose(*d))(o, 0, 2, 1, 3).reshape(B, S, D) @ wo

    def _B_ref(x, w1, b1, w2, b2):
        h = jnp.einsum("bsd,df->bsf", x, w1) + b1
        h = _gelu(h)
        return jnp.einsum("bsf,fd->bsd", h, w2) + b2

    x = A_x
    h = x + _A_ref(_layernorm(x, axis=-1), A_wqkv, A_wo)
    h2 = h + _B_ref(_layernorm(h, axis=-1), B_w1, B_b1, B_w2, B_b2)
    return h2
```

```python
import jax
import jax.numpy as jnp
from jax import lax
import jax.experimental.pallas as pl
import jax.experimental.pallas.tpu as pltpu

S = 2048
D = 512
H = 32
DH = 16
F = 1792
TQ = 512
NQ = S // TQ
CK = 128
NC = S // CK
TM = 512
NB = S // TM
EPS = 1e-5
QSCALE = (DH ** -0.5) * 1.4426950408889634

f32 = jnp.float32
bf16 = jnp.bfloat16


def _layernorm(x):
    m = jnp.mean(x, axis=-1, keepdims=True)
    xc = x - m
    v = jnp.mean(xc * xc, axis=-1, keepdims=True)
    return xc * lax.rsqrt(v + EPS)


def _kernel(x_ref, wqkv_ref, b1_ref, b2_ref, wo_hbm, w1_hbm, w2_hbm, o_ref,
            wo_ref, w1_ref, w2_ref, sem,
            k_ref, qt_ref, vt_ref, s_ref, m_ref, z_ref, ot_ref):
    step = pl.program_id(0)

    def weight_copies():
        return (pltpu.make_async_copy(wo_hbm, wo_ref, sem.at[0]),
                pltpu.make_async_copy(w1_hbm, w1_ref, sem.at[1]),
                pltpu.make_async_copy(w2_hbm, w2_ref, sem.at[2]))

    @pl.when(step == 0)
    def _attention():
        for cp in weight_copies():
            cp.start()

        wq_t = wqkv_ref[:, 0:D].astype(f32).T.astype(bf16)
        wv_t = wqkv_ref[:, 2 * D:3 * D].astype(f32).T.astype(bf16)
        wk = wqkv_ref[:, D:2 * D]
        nt = (((1,), (1,)), ((), ()))
        for b in range(NQ):
            xb = x_ref[b * TQ:(b + 1) * TQ, :].astype(f32)
            xn = _layernorm(xb).astype(bf16)
            kb = jnp.dot(xn, wk, preferred_element_type=f32).astype(bf16)
            for g in range(4):
                k_ref[g, b * TQ:(b + 1) * TQ, :] = kb[:, g * 128:(g + 1) * 128]
            qt = lax.dot_general(wq_t, xn, nt, preferred_element_type=f32)
            qt = (qt * QSCALE).astype(bf16)
            for g in range(4):
                qt_ref[b * 4 + g] = qt[g * 128:(g + 1) * 128, :]
            vt = lax.dot_general(wv_t, xn, nt, preferred_element_type=f32)
            vt_ref[:, b * TQ:(b + 1) * TQ] = vt.astype(bf16)

        z_ref[...] = jnp.zeros_like(z_ref)

        rowgrp = lax.broadcasted_iota(jnp.int32, (128, TQ), 0) // DH

        def stage(h_s, h_p):
            if h_s is not None:
                g = h_s // 8
                hh = h_s % 8
            if h_p is not None:
                row0 = h_p * DH
                if not isinstance(row0, int):
                    row0 = pl.multiple_of(row0, DH)
            for u in range(NQ):
                if h_s is not None:
                    q = qt_ref[u * 4 + g]
                    w = jnp.where(rowgrp == hh, q.astype(f32), 0.0).astype(bf16)
                    m_next = None
                if h_p is not None:
                    l = None
                    acc = z_ref[...]
                    m = m_ref[u]
                for c in range(NC):
                    if h_p is not None:
                        sp = s_ref[u, c * CK:(c + 1) * CK, :]
                    if h_s is not None:
                        s = jnp.dot(k_ref[g, c * CK:(c + 1) * CK, :], w,
                                    preferred_element_type=f32)
                        s_ref[u, c * CK:(c + 1) * CK, :] = s
                        for j in range(CK // 8):
                            sj = s[j * 8:(j + 1) * 8]
                            m_next = sj if m_next is None else jnp.maximum(m_next, sj)
                    if h_p is not None:
                        p = jnp.exp2(sp.reshape(CK // 8, 8, TQ) - m[None])
                        for j in reversed(range(CK // 16)):
                            t = p[2 * j] + p[2 * j + 1]
                            l = t if l is None else l + t
                        pb = p.reshape(CK, TQ).astype(bf16)
                        acc = acc + jnp.dot(
                            vt_ref[pl.ds(row0, DH), c * CK:(c + 1) * CK], pb,
                            preferred_element_type=f32)
                if h_p is not None:
                    lt = jnp.sum(l, axis=0, keepdims=True)
                    ot_ref[u, pl.ds(row0, DH), :] = acc / lt
                if h_s is not None:
                    mm = jnp.max(m_next, axis=0, keepdims=True)
                    m_ref[u] = jnp.broadcast_to(mm, (8, TQ))

        stage(0, None)

        def body(i, carry):
            stage(i + 1, i)
            return carry

        lax.fori_loop(0, H - 1, body, 0)
        stage(None, H - 1)

        for cp in weight_copies():
            cp.wait()

    r0 = pl.multiple_of(step * TM, TM)
    o = ot_ref[step].T.astype(bf16)
    attn = jnp.dot(o, wo_ref[...], preferred_element_type=f32)
    h = x_ref[pl.ds(r0, TM), :].astype(f32) + attn
    hn = _layernorm(h).astype(bf16)
    a = jnp.dot(hn, w1_ref[...], preferred_element_type=f32) + b1_ref[...].astype(f32)
    a = jax.nn.gelu(a, approximate=True).astype(bf16)
    y = jnp.dot(a, w2_ref[...], preferred_element_type=f32) + b2_ref[...].astype(f32)
    o_ref[...] = (h + y).astype(o_ref.dtype)


@jax.jit
def pallas_sequential_preLN__softmax_full_mha__dense_activation_gelu__prompt_kernel(
    A_x: jax.Array,
    A_wqkv: jax.Array,
    A_wo: jax.Array,
    B_x: jax.Array,
    B_w1: jax.Array,
    B_b1: jax.Array,
    B_w2: jax.Array,
    B_b2: jax.Array,
):
    del B_x
    x = A_x.reshape(S, D)
    b1 = B_b1.reshape(1, F)
    b2 = B_b2.reshape(1, D)

    def full(shape):
        return pl.BlockSpec(shape, lambda i: (0,) * len(shape))

    out = pl.pallas_call(
        _kernel,
        grid=(NB,),
        in_specs=[
            full((S, D)),
            full((D, 3 * D)),
            full((1, F)),
            full((1, D)),
            pl.BlockSpec(memory_space=pl.ANY),
            pl.BlockSpec(memory_space=pl.ANY),
            pl.BlockSpec(memory_space=pl.ANY),
        ],
        out_specs=pl.BlockSpec((TM, D), lambda i: (i, 0)),
        out_shape=jax.ShapeDtypeStruct((S, D), A_x.dtype),
        scratch_shapes=[
            pltpu.VMEM((D, D), bf16),
            pltpu.VMEM((D, F), bf16),
            pltpu.VMEM((F, D), bf16),
            pltpu.SemaphoreType.DMA((3,)),
            pltpu.VMEM((4, S, 128), bf16),
            pltpu.VMEM((NQ * 4, 128, TQ), bf16),
            pltpu.VMEM((D, S), bf16),
            pltpu.VMEM((NQ, S, TQ), f32),
            pltpu.VMEM((NQ, 8, TQ), f32),
            pltpu.VMEM((DH, TQ), f32),
            pltpu.VMEM((NQ, D, TQ), f32),
        ],
        compiler_params=pltpu.CompilerParams(
            dimension_semantics=("arbitrary",),
            vmem_limit_bytes=100 * 1024 * 1024,
        ),
    )(x, A_wqkv, b1, b2, A_wo, B_w1, B_w2)
    return out.reshape(1, S, D)
```

```python
import jax
import jax.numpy as jnp
from jax import lax
import jax.experimental.pallas as pl
import jax.experimental.pallas.tpu as pltpu

S = 2048
D = 512
H = 32
DH = 16
F = 1792
TQ = 512
NQ = S // TQ
CK = 128
NC = S // CK
TM = 512
NB = S // TM
EPS = 1e-5
QSCALE = (DH ** -0.5) * 1.4426950408889634

RO = 16
NM = CK - RO
NKB = NC * RO // 8
SEG = 4
SHIFT = 4
LAG = 2
L_LO = 2.0 ** -10
L_HI = 2.0 ** 64
F32_MAX = 3.0e38

f32 = jnp.float32
bf16 = jnp.bfloat16
i32 = jnp.int32
u32 = jnp.uint32


def _layernorm(x):
    m = jnp.mean(x, axis=-1, keepdims=True)
    xc = x - m
    v = jnp.mean(xc * xc, axis=-1, keepdims=True)
    return xc * lax.rsqrt(v + EPS)


def _vpu_plan():
    steps = [(u, c) for u in range(NQ) for c in range(NC)]
    segs = []
    for n, (u, c) in enumerate(steps):
        segs += [(n, (u, kb, d0))
                 for kb in range(c * RO // 8, (c + 1) * RO // 8)
                 for d0 in range(0, DH, SEG)]
    slots = [(n, j) for n in range(len(steps)) for j in range(NM // 8)]
    segpos = {}
    for i, (n, sg) in enumerate(segs):
        pos = (i * len(slots)) // len(segs) - SHIFT
        sl = slots[pos] if pos >= 0 else (0, -1)
        if sl[0] > n:
            sl = (n, NM // 8 - 1)
        segpos.setdefault(sl, []).append(sg)
    kbpos = {}
    for kb in range(NKB):
        kbpos.setdefault((kb * (len(steps) - 2)) // NKB, []).append(kb)
    return steps, segpos, kbpos


def _kernel(x_hbm, wqkv_hbm, wo_hbm, w1_hbm, w2_hbm, b1_ref, b2_ref, o_ref,
            x_ref, wq_ref, wk_ref, wv_ref, wo_ref, w1_ref, w2_ref, sem,
            xn_ref, k_ref, qt_ref, vt_ref, ko_ref, qba_ref, kba_ref, qbb_ref, kbb_ref,
            pc_ref, ac_ref, lc_ref, z_ref, zi_ref, zs_ref, bad_ref, ot_ref, s_ref):
    step = pl.program_id(0)

    def x_copy(b):
        return pltpu.make_async_copy(x_hbm.at[pl.ds(b * TQ, TQ), :],
                                     x_ref.at[pl.ds(b * TQ, TQ), :], sem.at[b])

    def w_copy(i):
        dst = (wq_ref, wk_ref, wv_ref)[i]
        return pltpu.make_async_copy(wqkv_hbm.at[:, pl.ds(i * D, D)], dst, sem.at[NQ + i])

    def late_copies():
        return (pltpu.make_async_copy(wo_hbm, wo_ref, sem.at[NQ + 3]),
                pltpu.make_async_copy(w1_hbm, w1_ref, sem.at[NQ + 4]),
                pltpu.make_async_copy(w2_hbm, w2_ref, sem.at[NQ + 5]))

    rowgrp = lax.broadcasted_iota(i32, (64, TQ), 0) // (DH // 2)

    def masked_q(u, h):
        q = qt_ref[u * 4 + h // 8]
        return pltpu.bitcast(jnp.where(rowgrp == h % 8, q, jnp.zeros_like(q)), bf16)

    def aligned(i, m):
        return i if isinstance(i, int) else pl.multiple_of(i, m)

    def make_kb(kb_ref, h, kb):
        kr = ko_ref[h // 8, kb * 8:(kb + 1) * 8, :]
        kr = pltpu.roll(kr, (128 - (h % 8) * DH) % 128, 1)
        for d in range(DH):
            kb_ref[d, kb * 8:(kb + 1) * 8, :] = jnp.broadcast_to(kr[:, d:d + 1], (8, 128))

    def make_qb(qb_ref, h, u):
        r0 = aligned((h % 8) * 8, 8)
        qh = pltpu.bitcast(qt_ref[u * 4 + h // 8, pl.ds(r0, 8), :], bf16).astype(f32)
        for d in range(DH):
            qb_ref[u, d] = jnp.broadcast_to(qh[d:d + 1, :], (8, TQ))

    @pl.when(step == 0)
    def _attention():
        x_copy(0).start()
        w_copy(1).start()

        z_ref[...] = jnp.zeros_like(z_ref)
        zi_ref[...] = jnp.zeros_like(zi_ref)
        bad_ref[...] = jnp.zeros_like(bad_ref)
        pc_ref[...] = jnp.zeros_like(pc_ref)
        ac_ref[...] = jnp.zeros_like(ac_ref)
        lc_ref[...] = jnp.ones_like(lc_ref)
        for i in range(NKB):
            zs_ref[i] = 0

        x_copy(0).wait()
        for b in range(1, NQ):
            x_copy(b).start()
        w_copy(0).start()
        w_copy(2).start()
        w_copy(1).wait()
        wk = wk_ref[...]
        for b in range(NQ):
            if b > 0:
                x_copy(b).wait()
            xn = _layernorm(x_ref[b * TQ:(b + 1) * TQ, :].astype(f32)).astype(bf16)
            xn_ref[b] = pltpu.bitcast(xn, u32)
            kb16 = jnp.dot(xn, wk, preferred_element_type=f32).astype(bf16)
            kpk = pltpu.bitcast(kb16, u32)
            for g in range(4):
                k_ref[g, b * TQ // 2:(b + 1) * TQ // 2, :] = kpk[:, g * 128:(g + 1) * 128]
                for cc in range(TQ // CK):
                    c = b * (TQ // CK) + cc
                    ko_ref[g, c * RO:(c + 1) * RO, :] = (
                        kb16[cc * CK + NM:(cc + 1) * CK, g * 128:(g + 1) * 128].astype(f32))
        w_copy(0).wait()
        w_copy(2).wait()
        for cp in late_copies():
            cp.start()
        wqv_t = jnp.concatenate(
            [wq_ref[...].astype(f32).T.astype(bf16), wv_ref[...].astype(f32).T.astype(bf16)],
            axis=0)
        nt = (((1,), (1,)), ((), ()))
        for kb in range(NKB):
            make_kb(kba_ref, 0, kb)
        for b in range(NQ):
            xn = pltpu.bitcast(xn_ref[b], bf16)
            qv = lax.dot_general(wqv_t, xn, nt, preferred_element_type=f32)
            qt = pltpu.bitcast((qv[0:D] * QSCALE).astype(bf16), u32)
            for g in range(4):
                qt_ref[b * 4 + g] = qt[g * 64:(g + 1) * 64, :]
            vt_ref[:, b * TQ:(b + 1) * TQ] = pltpu.bitcast(qv[D:2 * D].astype(bf16), u32)
            make_qb(qba_ref, 0, b)

        steps, segpos, kbpos = _vpu_plan()

        def do_pv(st, h, u, c, pb):
            r0 = aligned(h * 8, 8)
            vv = pltpu.bitcast(vt_ref[pl.ds(r0, 8), c * CK:(c + 1) * CK], bf16)
            st["acc"] = st["acc"] + jnp.dot(vv, pb, preferred_element_type=f32)
            if c == NC - 1:
                lt = jnp.sum(st["l"], axis=0, keepdims=True)
                o = st["acc"] * pl.reciprocal(lt, approx=False)
                ot_ref[u, pl.ds(aligned(h * DH, DH), DH), :] = o
                okl = jnp.logical_and(lt >= L_LO, lt <= L_HI)
                ok = jnp.logical_and(jnp.abs(o) <= F32_MAX, okl)
                bad_ref[...] = jnp.maximum(bad_ref[...], jnp.where(ok, 0.0, 1.0))

        def load_carry(hprev):
            st = dict(acc=ac_ref[...], l=lc_ref[...])
            return [(st, hprev, NQ - 1, NC - LAG + i, pltpu.bitcast(pc_ref[i], bf16))
                    for i in range(LAG)]

        def store_carry(pend):
            st = pend[0][0]
            ac_ref[...] = st["acc"]
            lc_ref[...] = st["l"]
            for i in range(LAG):
                pc_ref[i] = pltpu.bitcast(pend[i][4], u32)

        def head(h, qb_ref, kb_ref, hn, qbn_ref, kbn_ref):
            pend = load_carry(jnp.maximum(h - 1, 0))
            g = h // 8
            fmask = zi_ref[...] != 0
            sv = {}

            def run_segs(key, src):
                for (u2, kb, d0) in segpos.get(key, []):
                    for d in range(d0, d0 + SEG):
                        qb = qb_ref[u2 + zs_ref[kb], d]
                        kk = kb_ref[d, kb * 8:(kb + 1) * 8, :]
                        if d == d0 and src is not None:
                            kk = jnp.where(fmask, src, kk)
                        pr = jnp.concatenate([kk] * 4, axis=1) * qb
                        sv[u2, kb] = sv[u2, kb] + pr if (u2, kb) in sv else pr

            run_segs((0, -1), None)
            st = None
            for n, (u, c) in enumerate(steps):
                if c == 0:
                    st = dict(w=masked_q(u, h), l=None, acc=z_ref[...])
                lo = c * CK
                kk_ = pltpu.bitcast(k_ref[g, lo // 2:(lo + NM) // 2, :], bf16)
                s = jnp.dot(kk_, st["w"], preferred_element_type=f32)
                for j in range(NM // 8):
                    run_segs((n, j), s[j * 8:(j + 1) * 8, 0:128])
                    if j == 4:
                        for kb in kbpos.get(n, []):
                            make_kb(kbn_ref, hn, kb)
                s = jnp.concatenate(
                    [s] + [sv.pop((u, kb)) for kb in range(c * RO // 8, (c + 1) * RO // 8)],
                    axis=0)
                p = jnp.exp2(s).reshape(CK // 8, 8, TQ)
                for j in range(CK // 16):
                    t = p[2 * j] + p[2 * j + 1]
                    st["l"] = t if st["l"] is None else st["l"] + t
                pend.append((st, h, u, c, p.reshape(CK, TQ).astype(bf16)))
                do_pv(*pend.pop(0))
                if c == NC - 1:
                    make_qb(qbn_ref, hn, u)
            store_carry(pend)

        def body(i, carry):
            @pl.when(i % 2 == 0)
            def _():
                head(i, qba_ref, kba_ref, i + 1, qbb_ref, kbb_ref)

            @pl.when(i % 2 == 1)
            def _():
                head(i, qbb_ref, kbb_ref, jnp.minimum(i + 1, H - 1), qba_ref, kba_ref)
            return carry

        lax.fori_loop(0, H, body, 0)
        for item in load_carry(H - 1):
            do_pv(*item)

        @pl.when(jnp.max(bad_ref[...]) > 0.0)
        def _exact():
            def fb(t, carry):
                u = t // H
                h = t % H
                w = masked_q(u, h)

                def scores(cb, m):
                    kk = pltpu.bitcast(
                        k_ref[h // 8, pl.ds(pl.multiple_of(cb * 256, 256), 256), :], bf16)
                    s = jnp.dot(kk, w, preferred_element_type=f32)
                    s_ref[pl.ds(pl.multiple_of(cb * 512, 512), 512), :] = s
                    return jnp.maximum(m, jnp.max(s.reshape(64, 8, TQ), axis=0))

                m = lax.fori_loop(0, S // 512, scores, jnp.full((8, TQ), -jnp.inf, f32))
                m = jnp.max(m, axis=0, keepdims=True)

                def pv(cb, la):
                    l, acc = la
                    off = pl.multiple_of(cb * 512, 512)
                    p = jnp.exp2(s_ref[pl.ds(off, 512), :] - m)
                    l = l + jnp.sum(p.reshape(64, 8, TQ), axis=0)
                    vv = pltpu.bitcast(
                        vt_ref[pl.ds(pl.multiple_of(h * 8, 8), 8), pl.ds(off, 512)], bf16)
                    acc = acc + jnp.dot(vv, p.astype(bf16), preferred_element_type=f32)
                    return l, acc

                l, acc = lax.fori_loop(
                    0, S // 512, pv, (jnp.zeros((8, TQ), f32), jnp.zeros((DH, TQ), f32)))
                lt = jnp.sum(l, axis=0, keepdims=True)
                ot_ref[u, pl.ds(pl.multiple_of(h * DH, DH), DH), :] = (
                    acc * pl.reciprocal(lt, approx=False))
                return carry

            lax.fori_loop(0, NQ * H, fb, 0)

        for cp in late_copies():
            cp.wait()

    r0 = pl.multiple_of(step * TM, TM)
    o = ot_ref[step].T.astype(bf16)
    attn = jnp.dot(o, wo_ref[...], preferred_element_type=f32)
    h = x_ref[pl.ds(r0, TM), :].astype(f32) + attn
    hn = _layernorm(h).astype(bf16)
    a = jnp.dot(hn, w1_ref[...], preferred_element_type=f32) + b1_ref[...].astype(f32)[None, :]
    a = jax.nn.gelu(a, approximate=True).astype(bf16)
    y = jnp.dot(a, w2_ref[...], preferred_element_type=f32) + b2_ref[...].astype(f32)[None, :]
    o_ref[...] = (h + y).astype(o_ref.dtype)


@jax.jit
def pallas_sequential_preLN__softmax_full_mha__dense_activation_gelu__prompt_kernel(
    A_x: jax.Array,
    A_wqkv: jax.Array,
    A_wo: jax.Array,
    B_x: jax.Array,
    B_w1: jax.Array,
    B_b1: jax.Array,
    B_w2: jax.Array,
    B_b2: jax.Array,
):
    del B_x
    x = A_x.reshape(S, D)
    hbm = pl.BlockSpec(memory_space=pl.ANY)

    out = pl.pallas_call(
        _kernel,
        grid=(NB,),
        in_specs=[hbm, hbm, hbm, hbm, hbm,
                  pl.BlockSpec((F,), lambda i: (0,)),
                  pl.BlockSpec((D,), lambda i: (0,))],
        out_specs=pl.BlockSpec((TM, D), lambda i: (i, 0)),
        out_shape=jax.ShapeDtypeStruct((S, D), A_x.dtype),
        scratch_shapes=[
            pltpu.VMEM((S, D), bf16),
            pltpu.VMEM((D, D), bf16),
            pltpu.VMEM((D, D), bf16),
            pltpu.VMEM((D, D), bf16),
            pltpu.VMEM((D, D), bf16),
            pltpu.VMEM((D, F), bf16),
            pltpu.VMEM((F, D), bf16),
            pltpu.SemaphoreType.DMA((NQ + 6,)),
            pltpu.VMEM((NQ, TQ // 2, D), u32),
            pltpu.VMEM((4, S // 2, 128), u32),
            pltpu.VMEM((NQ * 4, 64, TQ), u32),
            pltpu.VMEM((D // 2, S), u32),
            pltpu.VMEM((4, NC * RO, 128), f32),
            pltpu.VMEM((NQ, DH, 8, TQ), f32),
            pltpu.VMEM((DH, NC * RO, 128), f32),
            pltpu.VMEM((NQ, DH, 8, TQ), f32),
            pltpu.VMEM((DH, NC * RO, 128), f32),
            pltpu.VMEM((LAG, CK // 2, TQ), u32),
            pltpu.VMEM((DH, TQ), f32),
            pltpu.VMEM((8, TQ), f32),
            pltpu.VMEM((DH, TQ), f32),
            pltpu.VMEM((8, 128), i32),
            pltpu.SMEM((NKB,), i32),
            pltpu.VMEM((DH, TQ), f32),
            pltpu.VMEM((NQ, D, TQ), f32),
            pltpu.VMEM((S, TQ), f32),
        ],
        compiler_params=pltpu.CompilerParams(
            dimension_semantics=("arbitrary",),
            vmem_limit_bytes=100 * 1024 * 1024,
        ),
    )(x, A_wqkv, A_wo, B_w1, B_w2, B_b1, B_b2)
    return out.reshape(1, S, D)
```

```python
import jax
import jax.numpy as jnp
from jax import lax
import jax.experimental.pallas as pl
import jax.experimental.pallas.tpu as pltpu

S = 2048
D = 512
H = 32
DH = 16
F = 1792
TQ = 512
NQ = S // TQ
CK = 128
NC = S // CK
TM = 512
NB = S // TM
NSUB = 2
TS = TM // NSUB
XCH = [(0, 256), (256, 256), (512, 512), (1024, 512), (1536, 512)]
NX = len(XCH)
EPS = 1e-5
QSCALE = (DH ** -0.5) * 1.4426950408889634

NV = [(1, 1, 1, 2)[c % 4] for c in range(NC)]
KB0 = [2 * sum(NV[:c]) for c in range(NC + 1)]
NKB = KB0[NC]
RV = NKB * 8
RPAD = 384
SEG = 4
SHIFT = 4
LAGG = 9
KG = 10
L_LO = 2.0 ** -10
L_HI = 2.0 ** 64
V_HI = 2.0 ** 60

f32 = jnp.float32
bf16 = jnp.bfloat16
i32 = jnp.int32
u32 = jnp.uint32


def _layernorm(x):
    m = jnp.mean(x, axis=-1, keepdims=True)
    xc = x - m
    v = jnp.mean(xc * xc, axis=-1, keepdims=True)
    return xc * lax.rsqrt(v + EPS)


class _Plan:
    def __init__(self):
        kstream = [(c, g) for c in range(NC) for g in range(7, NV[c] - 1, -1)]
        self.ng = len(kstream)
        self.kpos = {cg: i for i, cg in enumerate(kstream)}
        self.stream = [(u, c, g) for u in range(NQ) for (c, g) in kstream]
        ns = self.ns = len(self.stream)
        self.last = {}
        for x, (u, c, g) in enumerate(self.stream):
            self.last[u, c] = x
        tiles = [(u, c) for u in range(NQ) for c in range(NC)]
        self.pv_after, self.carry = {}, []
        for t in tiles:
            x = self.last[t] + LAGG
            if x <= ns - 1:
                self.pv_after.setdefault(x, []).append(t)
            else:
                self.carry.append((t, x - ns))
        assert all(t[0] == NQ - 1 for t, _ in self.carry)
        cuts = set(self.pv_after) | {x for _, x in self.carry} | {
            x for x in range(ns) if x == ns - 1 or self.stream[x + 1][0] != self.stream[x][0]}
        self.pieces, x0 = [], 0
        for x in range(ns):
            if x in cuts:
                self.pieces.append((x0, x + 1))
                x0 = x + 1
        segs = [(t, kb, d0) for t in tiles for kb in range(KB0[t[1]], KB0[t[1] + 1])
                for d0 in range(0, DH, SEG)]
        self.segpos = {}
        for i, (t, kb, d0) in enumerate(segs):
            pos = min((i * 2 * ns) // len(segs) - SHIFT, 2 * self.last[t] + 1)
            self.segpos.setdefault(max(pos, -1), []).append((t[0], kb, d0))
        items = [(u, d) for u in range(NQ) for d in range(DH)]
        self.qbpos = {}
        for i, it in enumerate(items):
            self.qbpos.setdefault((i * (ns - 8)) // len(items), []).append(it)
        self.kbpos = {}
        for kb in range(0, NKB, KG):
            self.kbpos.setdefault(8 + (kb * (ns - 30 - 6 * KG)) // NKB, []).append(kb)


PLAN = _Plan()
NCARRY = len(PLAN.carry)


def _kernel(x_hbm, wqkv_hbm, wo_hbm, w1_hbm, w2_hbm, b1_hbm, b2_hbm, o_hbm,
            x_ref, wq_ref, wk_ref, wv_ref, wo_ref, w1_ref, w2_ref, sem,
            xn_ref, k_ref, qt_ref, vt_ref, ko_ref,
            qba_ref, kba_ref, kra_ref, qbb_ref, kbb_ref, krb_ref,
            pc_ref, misc_ref, zi_ref, zs_ref, ot_ref, l_ref, ob_ref, s_ref, bias_ref, o_ref, osem):
    step = pl.program_id(0)
    P = PLAN
    AC, ZR, VM, LC = slice(0, 16), slice(16, 32), slice(32, 40), slice(48, 56)

    def x_copy(i):
        r0, n = XCH[i]
        return pltpu.make_async_copy(x_hbm.at[pl.ds(r0, n), :], x_ref.at[pl.ds(r0, n), :],
                                     sem.at[i])

    def w_copy(i):
        dst = (wq_ref, wk_ref, wv_ref)[i]
        return pltpu.make_async_copy(wqkv_hbm.at[:, pl.ds(i * D, D)], dst, sem.at[NX + i])

    def late_copies():
        return (pltpu.make_async_copy(wo_hbm, wo_ref, sem.at[NX + 3]),
                pltpu.make_async_copy(w1_hbm, w1_ref, sem.at[NX + 4]),
                pltpu.make_async_copy(w2_hbm, w2_ref, sem.at[NX + 5]),
                pltpu.make_async_copy(b1_hbm, bias_ref.at[pl.ds(0, F)], sem.at[NX + 6]),
                pltpu.make_async_copy(b2_hbm, bias_ref.at[pl.ds(2048, D)], sem.at[NX + 7]))

    def aligned(i, m):
        return i if isinstance(i, int) else pl.multiple_of(i, m)

    def head_shift(h):
        return (128 - (h % 8) * DH) % 128

    def q_rows(h, u):
        return qt_ref[u * 4 + h // 8, pl.ds(aligned((h % 8) * 8, 8), 8), :]

    def q_weights(h, u):
        q16 = pltpu.bitcast(q_rows(h, u), bf16)
        return jnp.concatenate([q16, jnp.zeros((128 - DH, TQ), bf16)], axis=0)

    def roll_ko(h):
        return pltpu.roll(ko_ref[h // 8, 0:RV, :], head_shift(h), 1)

    def make_kb(kb_ref, kro, kb, tie=None):
        kr = kro[kb * 8:(kb + KG) * 8, :]
        if tie is not None:
            kr = jnp.concatenate([tie(kr[i * 8:(i + 1) * 8]) for i in range(KG)], axis=0)
        for d in range(DH):
            kb_ref[kb:kb + KG, d * 8:(d + 1) * 8, :] = jnp.broadcast_to(
                kr[:, d:d + 1], (8 * KG, 128)).reshape(KG, 8, 128)

    def make_kr(kr_ref, h, c):
        kk = k_ref[h // 8, c * 64 + 8 * NV[c]:(c + 1) * 64, :]
        kk = pltpu.roll(kk, head_shift(h), 1)
        for g in range(NV[c], 8):
            i = P.kpos[c, g]
            kr_ref[i * 8:(i + 1) * 8, :] = kk[(g - NV[c]) * 8:(g - NV[c] + 1) * 8]

    def o_block(u, i):
        linv = 1.0 / l_ref[u, :, i * TS:(i + 1) * TS]
        o = jnp.concatenate(
            [ot_ref[u, h * DH:(h + 1) * DH, i * TS:(i + 1) * TS] * linv[h:h + 1, :]
             for h in range(H)], axis=0)
        return o.T.astype(bf16)

    @pl.when(step == 0)
    def _attention():
        x_copy(0).start()
        w_copy(1).start()
        for i in range(1, NX):
            x_copy(i).start()
        w_copy(0).start()
        w_copy(2).start()

        misc_ref[0:32, :] = jnp.zeros((32, TQ), f32)
        misc_ref[LC, :] = jnp.ones((8, TQ), f32)
        zi_ref[0:8, :] = jnp.zeros((8, 128), i32)
        pc_ref[...] = jnp.zeros_like(pc_ref)
        for i in range(NKB):
            zs_ref[i] = 0

        def ln_chunk(r0, n, pace=None):
            x = x_ref[r0:r0 + n, :].astype(f32)
            if pace is not None:
                fm = zi_ref[0:8, :] != 0
                m, nj = pace.shape[0] // 8, n // 8
                parts = []
                for j in range(nj):
                    pr, pc = (j * 3 * m) // nj % m, (j * 3) // nj
                    parts.append(jnp.where(fm, pace[pr * 8:pr * 8 + 8, pc * 128:pc * 128 + 128],
                                           x[j * 8:(j + 1) * 8, 0:128]))
                x0 = jnp.concatenate(parts, axis=0)
                x = jnp.concatenate([x0, x[:, 128:]], axis=1)
            xn_ref[r0 // 2:(r0 + n) // 2, :] = pltpu.bitcast(_layernorm(x).astype(bf16), u32)

        def k_chunk(r0, n):
            xn = pltpu.bitcast(xn_ref[r0 // 2:(r0 + n) // 2, :], bf16)
            kf = jnp.dot(xn, wk_ref[...], preferred_element_type=f32)
            kb16 = kf.astype(bf16)
            kpk = pltpu.bitcast(kb16, u32)
            for g in range(4):
                k_ref[g, r0 // 2:(r0 + n) // 2, :] = kpk[:, g * 128:(g + 1) * 128]
                for cc in range(n // CK):
                    c = r0 // CK + cc
                    ko_ref[g, KB0[c] * 8:KB0[c + 1] * 8, :] = (
                        kb16[cc * CK:cc * CK + 16 * NV[c], g * 128:(g + 1) * 128].astype(f32))
            return kf

        x_copy(0).wait()
        ln_chunk(0, 256)
        w_copy(1).wait()
        x_copy(1).wait()
        ln_chunk(256, 256, k_chunk(0, 256))
        x_copy(2).wait()
        ln_chunk(512, 512, k_chunk(256, 256))
        x_copy(3).wait()
        kf = k_chunk(512, 512)
        ln_chunk(1024, 256)
        ln_chunk(1280, 256, kf)
        k_chunk(1024, 256)
        x_copy(4).wait()
        w_copy(0).wait()
        w_copy(2).wait()
        for cp in late_copies():
            cp.start()
        k_chunk(1280, 256)
        ln_chunk(1536, 512)
        k_chunk(1536, 512)
        wqv_t = jnp.concatenate(
            [wq_ref[...].astype(f32).T.astype(bf16), wv_ref[...].astype(f32).T.astype(bf16)],
            axis=0)
        nt = (((1,), (1,)), ((), ()))
        kro0 = roll_ko(0)
        for kb in range(0, NKB, KG):
            make_kb(kba_ref, kro0, kb)
        for c in range(NC):
            make_kr(kra_ref, 0, c)
        for b in range(NQ):
            xn = pltpu.bitcast(xn_ref[b * TQ // 2:(b + 1) * TQ // 2, :], bf16)
            qv = lax.dot_general(wqv_t, xn, nt, preferred_element_type=f32)
            qt = pltpu.bitcast((qv[0:D] * QSCALE).astype(bf16), u32)
            for g in range(4):
                qt_ref[b * 4 + g] = qt[g * 64:(g + 1) * 64, :]
            vt_ref[:, b * TQ:(b + 1) * TQ] = pltpu.bitcast(qv[D:2 * D].astype(bf16), u32)
            va = jnp.max(jnp.abs(qv[D:2 * D]).reshape(D // 8, 8, TQ), axis=0)
            vmax = va if b == 0 else jnp.maximum(vmax, va)
            qh = pltpu.bitcast(q_rows(0, b), bf16).astype(f32)
            for d in range(DH):
                qba_ref[b, d * 8:(d + 1) * 8, :] = jnp.broadcast_to(qh[d:d + 1, :], (8, TQ))

        misc_ref[VM, :] = vmax

        def do_pv(st, h, u, c, p):
            vv = pltpu.bitcast(vt_ref[pl.ds(aligned(h * 8, 8), 8), c * CK:(c + 1) * CK], bf16)
            st["acc"] = st["acc"] + lax.dot_general(
                vv, p, (((1,), (0,)), ((), ())), precision=lax.Precision.DEFAULT,
                preferred_element_type=f32)
            if c == NC - 1:
                ot_ref[u, pl.ds(aligned(h * DH, DH), DH), :] = st["acc"]
                l_ref[u, pl.ds(h, 1), :] = jnp.sum(st["l"], axis=0, keepdims=True)

        def carried(hprev):
            st = dict(acc=misc_ref[AC, :], l=misc_ref[LC, :])
            return {x: (st, hprev, t[0], t[1], pc_ref[i]) for i, (t, x) in enumerate(P.carry)}

        def head(h, qb_ref, kb_ref, kr_ref, hn, qbn_ref, kbn_ref, krn_ref):
            cpend = carried(jnp.maximum(h - 1, 0))
            fmask = zi_ref[0:8, :] != 0
            fmask4 = jnp.concatenate([fmask] * 4, axis=1)
            st, sv, pg, qhn, ptile, uidx = {}, {}, {}, {}, {}, {}

            def finish_group(u, c, g, s16):
                p = jnp.exp2(s16)
                t = p[0:8] + p[8:16]
                st[u]["l"] = t if st[u]["l"] is None else st[u]["l"] + t
                pg[u, c, g] = p

            def run_segs(key, src):
                for (u2, kb, d0) in P.segpos.get(key, []):
                    if d0 == 0:
                        uidx[u2, kb] = u2 + zs_ref[kb]
                    qb = qb_ref[uidx[u2, kb], d0 * 8:(d0 + SEG) * 8, :]
                    kk = kb_ref[kb, d0 * 8:(d0 + SEG) * 8, :]
                    if src is not None:
                        kk = jnp.concatenate([lax.select(fmask, src, kk[0:8]), kk[8:]], axis=0)
                    pr = jnp.concatenate([kk] * 4, axis=1) * qb
                    for d in range(SEG):
                        t = pr[d * 8:(d + 1) * 8]
                        sv[u2, kb] = sv[u2, kb] + t if (u2, kb) in sv else t

            kro = roll_ko(hn)
            for c in range(NC):
                make_kr(krn_ref, hn, c)
            run_segs(-1, None)
            for (x0, x1) in P.pieces:
                u = P.stream[x0][0]
                if u not in st:
                    st[u] = dict(w=q_weights(h, u), l=None, acc=misc_ref[ZR, :])
                i0 = x0 - u * P.ng
                kk_ = pltpu.bitcast(kr_ref[i0 * 8:(i0 + x1 - x0) * 8, :], bf16)
                s = jnp.dot(kk_, st[u]["w"], preferred_element_type=f32)
                for x in range(x0, x1):
                    _, c, g = P.stream[x]
                    r = (x - x0) * 16
                    for half in range(2):
                        if 2 * x + half in P.segpos:
                            run_segs(2 * x + half, s[r + 8 * half:r + 8 * half + 8, 0:128])
                    finish_group(u, c, g, s[r:r + 16])
                    for (u3, d3) in P.qbpos.get(x, []):
                        if u3 not in qhn:
                            qhn[u3] = pltpu.bitcast(q_rows(hn, u3), bf16).astype(f32)
                        val = jnp.broadcast_to(qhn[u3][d3:d3 + 1, :], (8, TQ))
                        qbn_ref[u3, d3 * 8:(d3 + 1) * 8, :] = lax.select(fmask4, s[r:r + 8], val)
                    for kb in P.kbpos.get(x, []):
                        make_kb(kbn_ref, kro, kb,
                                lambda v, src=s[r:r + 8, 128:256]: lax.select(fmask, src, v))
                    if x == P.last[u, c]:
                        for g2 in range(NV[c]):
                            kb = KB0[c] + 2 * g2
                            finish_group(u, c, g2, jnp.concatenate(
                                [sv.pop((u, kb)), sv.pop((u, kb + 1))], axis=0))
                        ptile[u, c] = jnp.concatenate(
                            [pg.pop((u, c, g2)) for g2 in range(8)], axis=0)
                if x1 - 1 in cpend:
                    do_pv(*cpend.pop(x1 - 1))
                for t in P.pv_after.get(x1 - 1, []):
                    do_pv(st[t[0]], h, t[0], t[1], ptile.pop(t))
            misc_ref[AC, :] = st[NQ - 1]["acc"]
            misc_ref[LC, :] = st[NQ - 1]["l"]
            for i, (t, _) in enumerate(P.carry):
                pc_ref[i] = ptile.pop(t)

        def body(i, carry):
            @pl.when(i % 2 == 0)
            def _():
                head(i, qba_ref, kba_ref, kra_ref, i + 1, qbb_ref, kbb_ref, krb_ref)

            @pl.when(i % 2 == 1)
            def _():
                head(i, qbb_ref, kbb_ref, krb_ref, jnp.minimum(i + 1, H - 1),
                     qba_ref, kba_ref, kra_ref)
            return carry

        lax.fori_loop(0, H, body, 0)
        for item in carried(H - 1).values():
            do_pv(*item)
        ob_ref[...] = pltpu.bitcast(o_block(0, 0), u32)

        lall = l_ref[...].reshape(NQ * H, TQ)
        bad_l = jnp.where(jnp.logical_and(lall >= L_LO, lall <= L_HI), 0.0, 1.0)
        bad_v = jnp.where(misc_ref[VM, :] <= V_HI, 0.0, 1.0)
        bad = jnp.maximum(jnp.max(bad_l.reshape(NQ * H // 8, 8, TQ), axis=0), bad_v)

        @pl.when(jnp.max(bad) > 0.0)
        def _exact():
            rowgrp = lax.broadcasted_iota(i32, (64, TQ), 0) // (DH // 2)

            def fb(t, carry):
                u = t // H
                h = t % H
                q = qt_ref[u * 4 + h // 8]
                w = pltpu.bitcast(jnp.where(rowgrp == h % 8, q, jnp.zeros_like(q)), bf16)

                def scores(cb, m):
                    kk = pltpu.bitcast(
                        k_ref[h // 8, pl.ds(pl.multiple_of(cb * 256, 256), 256), :], bf16)
                    s = jnp.dot(kk, w, preferred_element_type=f32)
                    s_ref[pl.ds(pl.multiple_of(cb * 512, 512), 512), :] = s
                    return jnp.maximum(m, jnp.max(s.reshape(64, 8, TQ), axis=0))

                m = lax.fori_loop(0, S // 512, scores, jnp.full((8, TQ), -jnp.inf, f32))
                m = jnp.max(m, axis=0, keepdims=True)

                def pv(cb, la):
                    l, acc = la
                    off = pl.multiple_of(cb * 512, 512)
                    p = jnp.exp2(s_ref[pl.ds(off, 512), :] - m)
                    l = l + jnp.sum(p.reshape(64, 8, TQ), axis=0)
                    vv = pltpu.bitcast(
                        vt_ref[pl.ds(pl.multiple_of(h * 8, 8), 8), pl.ds(off, 512)], bf16)
                    acc = acc + jnp.dot(vv, p.astype(bf16), preferred_element_type=f32)
                    return l, acc

                l, acc = lax.fori_loop(
                    0, S // 512, pv, (jnp.zeros((8, TQ), f32), jnp.zeros((DH, TQ), f32)))
                ot_ref[u, pl.ds(pl.multiple_of(h * DH, DH), DH), :] = acc
                l_ref[u, pl.ds(h, 1), :] = jnp.sum(l, axis=0, keepdims=True)
                return carry

            lax.fori_loop(0, NQ * H, fb, 0)
            ob_ref[...] = pltpu.bitcast(o_block(0, 0), u32)

        for cp in late_copies():
            cp.wait()

    b1 = bias_ref[0:F].astype(f32)[None, :]
    b2 = bias_ref[2048:2048 + D].astype(f32)[None, :]

    def out_copy(j):
        return pltpu.make_async_copy(o_ref.at[j], o_hbm.at[pl.ds(aligned(j * TS, TS), TS), :],
                                     osem.at[j])

    hs, hns = [], []
    for i in range(NSUB):
        r0 = pl.multiple_of(step * TM + i * TS, TS)
        o = pltpu.bitcast(ob_ref[...], bf16) if i == 0 else o_block(step, i)
        attn = jnp.dot(o, wo_ref[...], preferred_element_type=f32)
        h = x_ref[pl.ds(r0, TS), :].astype(f32) + attn
        hs.append(h)
        hns.append(_layernorm(h).astype(bf16))
    for i in range(NSUB):
        a = jnp.dot(hns[i], w1_ref[...], preferred_element_type=f32) + b1
        a = jax.nn.gelu(a, approximate=True).astype(bf16)
        y = jnp.dot(a, w2_ref[...], preferred_element_type=f32) + b2
        o_ref[step * NSUB + i] = (hs[i] + y).astype(o_ref.dtype)
        out_copy(step * NSUB + i).start()
    ob_ref[...] = pltpu.bitcast(o_block(jnp.minimum(step + 1, NB - 1), 0), u32)

    @pl.when(step == NB - 1)
    def _():
        for j in range(NB * NSUB):
            out_copy(j).wait()


@jax.jit
def pallas_sequential_preLN__softmax_full_mha__dense_activation_gelu__prompt_kernel(
    A_x: jax.Array,
    A_wqkv: jax.Array,
    A_wo: jax.Array,
    B_x: jax.Array,
    B_w1: jax.Array,
    B_b1: jax.Array,
    B_w2: jax.Array,
    B_b2: jax.Array,
):
    del B_x
    x = A_x.reshape(S, D)
    hbm = pl.BlockSpec(memory_space=pl.ANY)
    tables = [
        pltpu.VMEM((NQ, DH * 8, TQ), f32),
        pltpu.VMEM((RPAD // 8, DH * 8, 128), f32),
        pltpu.VMEM((1024, 128), u32),
    ]

    out = pl.pallas_call(
        _kernel,
        grid=(NB,),
        in_specs=[hbm] * 7,
        out_specs=hbm,
        out_shape=jax.ShapeDtypeStruct((S, D), A_x.dtype),
        scratch_shapes=[
            pltpu.VMEM((S, D), bf16),
            pltpu.VMEM((D, D), bf16),
            pltpu.VMEM((D, D), bf16),
            pltpu.VMEM((D, D), bf16),
            pltpu.VMEM((D, D), bf16),
            pltpu.VMEM((D, F), bf16),
            pltpu.VMEM((F, D), bf16),
            pltpu.SemaphoreType.DMA((NX + 8,)),
            pltpu.VMEM((S // 2, D), u32),
            pltpu.VMEM((4, S // 2, 128), u32),
            pltpu.VMEM((NQ * 4, 64, TQ), u32),
            pltpu.VMEM((D // 2, S), u32),
            pltpu.VMEM((4, RPAD, 128), f32),
        ] + tables + tables + [
            pltpu.VMEM((NCARRY, CK, TQ), f32),
            pltpu.VMEM((64, TQ), f32),
            pltpu.VMEM((128, 128), i32),
            pltpu.SMEM((NKB,), i32),
            pltpu.VMEM((NQ, D, TQ), f32),
            pltpu.VMEM((NQ, H, TQ), f32),
            pltpu.VMEM((TS // 2, D), u32),
            pltpu.VMEM((S, TQ), f32),
            pltpu.VMEM((32768,), bf16),
            pltpu.VMEM((S // TS, TS, D), bf16),
            pltpu.SemaphoreType.DMA((S // TS,)),
        ],
        compiler_params=pltpu.CompilerParams(
            dimension_semantics=("arbitrary",),
            vmem_limit_bytes=100 * 1024 * 1024,
        ),
    )(x, A_wqkv, A_wo, B_w1, B_w2, B_b1, B_b2)
    return out.reshape(1, S, D)
```

```python
import jax
import jax.numpy as jnp
from jax import lax
import jax.experimental.pallas as pl
import jax.experimental.pallas.tpu as pltpu

S = 2048
D = 512
H = 32
DH = 16
F = 1792
TQ = 512
NQ = S // TQ
CK = 128
NC = S // CK
TM = 512
NB = S // TM
NSUB = 2
TS = TM // NSUB
XCH = [(0, 256), (256, 256), (512, 512), (1024, 512), (1536, 512)]
NX = len(XCH)
EPS = 1e-5
QSCALE = (DH ** -0.5) * 1.4426950408889634

NV = [2 + c % 2 for c in range(NC)]
KB0 = [sum(NV[:c]) for c in range(NC + 1)]
MB0 = [16 * c - KB0[c] for c in range(NC + 1)]
NKB = KB0[NC]
RV = NKB * 8
RPAD = 384
SEG = 4
SHIFT = 2
LAGG = 8
KBX = 8
L_LO = 2.0 ** -10
L_HI = 2.0 ** 64
V_HI = 2.0 ** 60

f32 = jnp.float32
bf16 = jnp.bfloat16
i32 = jnp.int32
u32 = jnp.uint32


def _layernorm(x):
    m = jnp.mean(x, axis=-1, keepdims=True)
    xc = x - m
    v = jnp.mean(xc * xc, axis=-1, keepdims=True)
    return xc * lax.rsqrt(v + EPS)


class _Plan:
    def __init__(self):
        blocks = [(c, b) for c in range(NC) for b in range(15, NV[c] - 1, -1)]
        assert len(blocks) % 2 == 0
        self.ng = len(blocks) // 2
        self.stream = [(u, blocks[2 * i], blocks[2 * i + 1])
                       for u in range(NQ) for i in range(self.ng)]
        ns = self.ns = len(self.stream)
        self.last, self.lasth = {}, {}
        for x, (u, b0, b1) in enumerate(self.stream):
            for half, (c, b) in enumerate((b0, b1)):
                self.last[u, c] = x
                self.lasth[u, c] = 2 * x + half
        tiles = [(u, c) for u in range(NQ) for c in range(NC)]
        self.pv_after, self.carry = {}, []
        for t in tiles:
            x = self.last[t] + LAGG
            if x <= ns - 1:
                self.pv_after.setdefault(x, []).append(t)
            else:
                self.carry.append((t, x - ns))
        assert all(t[0] == NQ - 1 for t, _ in self.carry)
        cuts = set(self.pv_after) | {x for _, x in self.carry} | {
            x for x in range(ns) if x == ns - 1 or self.stream[x + 1][0] != self.stream[x][0]}
        self.pieces, x0 = [], 0
        for x in range(ns):
            if x in cuts:
                self.pieces.append((x0, x + 1))
                x0 = x + 1
        segs = [(t, kb, d0) for t in tiles for kb in range(KB0[t[1]], KB0[t[1] + 1])
                for d0 in range(0, DH, SEG)]
        self.segpos = {}
        for i, (t, kb, d0) in enumerate(segs):
            pos = min((i * 2 * ns) // len(segs) - SHIFT, self.lasth[t])
            self.segpos.setdefault(max(pos, -1), []).append((t[0], kb, d0))
        items = [(u, d) for u in range(NQ) for d in range(DH)]
        self.qbpos = {}
        for i, it in enumerate(items):
            self.qbpos.setdefault((i * (ns - 8)) // len(items), []).append(it)


PLAN = _Plan()
NCARRY = len(PLAN.carry)


def _kernel(x_hbm, wqkv_hbm, wo_hbm, w1_hbm, w2_hbm, b1_hbm, b2_hbm, o_hbm,
            x_ref, wq_ref, wk_ref, wv_ref, wo_ref, w1_ref, w2_ref, sem,
            xn_ref, k_ref, ks_ref, qt_ref, vt_ref, ko_ref,
            qba_ref, kba_ref, kra_ref, qbb_ref, kbb_ref, krb_ref,
            pc_ref, misc_ref, zi_ref, zs_ref, ot_ref, l_ref, ob_ref, s_ref, bias_ref, o_ref, osem):
    step = pl.program_id(0)
    P = PLAN
    AC, ZR, VM, LC = slice(0, 16), slice(16, 32), slice(32, 40), slice(48, 56)
    KL = slice(56, 64)

    def x_copy(i):
        r0, n = XCH[i]
        return pltpu.make_async_copy(x_hbm.at[pl.ds(r0, n), :], x_ref.at[pl.ds(r0, n), :],
                                     sem.at[i])

    def w_copy(i):
        dst = (wq_ref, wk_ref, wv_ref)[i]
        return pltpu.make_async_copy(wqkv_hbm.at[:, pl.ds(i * D, D)], dst, sem.at[NX + i])

    def late_copies():
        return (pltpu.make_async_copy(wo_hbm, wo_ref, sem.at[NX + 3]),
                pltpu.make_async_copy(w1_hbm, w1_ref, sem.at[NX + 4]),
                pltpu.make_async_copy(w2_hbm, w2_ref, sem.at[NX + 5]),
                pltpu.make_async_copy(b1_hbm, bias_ref.at[pl.ds(0, F)], sem.at[NX + 6]),
                pltpu.make_async_copy(b2_hbm, bias_ref.at[pl.ds(2048, D)], sem.at[NX + 7]))

    def aligned(i, m):
        return i if isinstance(i, int) else pl.multiple_of(i, m)

    def head_shift(h):
        return (128 - (h % 8) * DH) % 128

    def q_rows(h, u):
        return qt_ref[u * 4 + h // 8, pl.ds(aligned((h % 8) * 8, 8), 8), :]

    def q_weights(h, u):
        q16 = pltpu.bitcast(q_rows(h, u), bf16)
        return jnp.concatenate([q16, jnp.zeros((128 - DH, TQ), bf16)], axis=0)

    def roll_ko(h):
        return pltpu.roll(ko_ref[h // 8, 0:RV, :], head_shift(h), 1)

    def make_kb(kb_ref, kro):
        for d in range(DH):
            kb_ref[0:NKB, d * 8:(d + 1) * 8, :] = jnp.broadcast_to(
                kro[:, d:d + 1], (RV, 128)).reshape(NKB, 8, 128)

    def make_kr(kr_ref, h):
        kr_ref[0:P.ng * 8, :] = pltpu.roll(ks_ref[h // 8, 0:P.ng * 8, :], head_shift(h), 1)

    def o_block(u, i):
        linv = 1.0 / l_ref[u, :, i * TS:(i + 1) * TS]
        o = jnp.concatenate(
            [ot_ref[u, h * DH:(h + 1) * DH, i * TS:(i + 1) * TS] * linv[h:h + 1, :]
             for h in range(H)], axis=0)
        return o.T.astype(bf16)

    @pl.when(step == 0)
    def _attention():
        x_copy(0).start()
        w_copy(1).start()
        for i in range(1, NX):
            x_copy(i).start()
        w_copy(0).start()
        w_copy(2).start()

        misc_ref[0:32, :] = jnp.zeros((32, TQ), f32)
        misc_ref[LC, :] = jnp.ones((8, TQ), f32)
        zi_ref[0:8, :] = jnp.zeros((8, 128), i32)
        pc_ref[...] = jnp.zeros_like(pc_ref)
        for i in range(NKB):
            zs_ref[i] = 0

        def ln_chunk(r0, n, pace=None):
            x = x_ref[r0:r0 + n, :].astype(f32)
            if pace is not None:
                fm = zi_ref[0:8, :] != 0
                m, nj = pace.shape[0] // 8, n // 8
                parts = []
                for j in range(nj):
                    pr, pc = (j * 3 * m) // nj % m, (j * 3) // nj
                    parts.append(jnp.where(fm, pace[pr * 8:pr * 8 + 8, pc * 128:pc * 128 + 128],
                                           x[j * 8:(j + 1) * 8, 0:128]))
                x0 = jnp.concatenate(parts, axis=0)
                x = jnp.concatenate([x0, x[:, 128:]], axis=1)
            xn_ref[r0 // 2:(r0 + n) // 2, :] = pltpu.bitcast(_layernorm(x).astype(bf16), u32)

        def k_chunk(r0, n):
            xn = pltpu.bitcast(xn_ref[r0 // 2:(r0 + n) // 2, :], bf16)
            kf = jnp.dot(xn, wk_ref[...], preferred_element_type=f32)
            kb16 = kf.astype(bf16)
            kpk = pltpu.bitcast(kb16, u32)
            c0, c1 = r0 // CK, (r0 + n) // CK
            blks = [kf[(c - c0) * CK + b * 8:(c - c0) * CK + b * 8 + 8]
                    for c in range(c0, c1) for b in range(15, NV[c] - 1, -1)]
            if MB0[c0] % 2:
                blks = [misc_ref[KL, :]] + blks
            if MB0[c1] % 2:
                misc_ref[KL, :] = blks.pop()
            kspk = pltpu.bitcast(jnp.concatenate(blks, axis=0).astype(bf16), u32)
            kof = jnp.concatenate(
                [kf[(c - c0) * CK:(c - c0) * CK + 8 * NV[c]] for c in range(c0, c1)], axis=0)
            kof = kof.astype(bf16).astype(f32)
            for g in range(4):
                k_ref[g, r0 // 2:(r0 + n) // 2, :] = kpk[:, g * 128:(g + 1) * 128]
                ks_ref[g, MB0[c0] // 2 * 8:MB0[c1] // 2 * 8, :] = kspk[:, g * 128:(g + 1) * 128]
                ko_ref[g, KB0[c0] * 8:KB0[c1] * 8, :] = kof[:, g * 128:(g + 1) * 128]
            return kf

        x_copy(0).wait()
        ln_chunk(0, 256)
        w_copy(1).wait()
        x_copy(1).wait()
        ln_chunk(256, 256, k_chunk(0, 256))
        x_copy(2).wait()
        ln_chunk(512, 512, k_chunk(256, 256))
        x_copy(3).wait()
        kf = k_chunk(512, 512)
        ln_chunk(1024, 256)
        ln_chunk(1280, 256, kf)
        k_chunk(1024, 256)
        x_copy(4).wait()
        w_copy(0).wait()
        w_copy(2).wait()
        for cp in late_copies():
            cp.start()
        k_chunk(1280, 256)
        ln_chunk(1536, 512)
        k_chunk(1536, 512)
        wqv_t = jnp.concatenate(
            [wq_ref[...].astype(f32).T.astype(bf16), wv_ref[...].astype(f32).T.astype(bf16)],
            axis=0)
        nt = (((1,), (1,)), ((), ()))
        make_kb(kba_ref, roll_ko(0))
        make_kr(kra_ref, 0)
        for b in range(NQ):
            xn = pltpu.bitcast(xn_ref[b * TQ // 2:(b + 1) * TQ // 2, :], bf16)
            qv = lax.dot_general(wqv_t, xn, nt, preferred_element_type=f32)
            qt = pltpu.bitcast((qv[0:D] * QSCALE).astype(bf16), u32)
            for g in range(4):
                qt_ref[b * 4 + g] = qt[g * 64:(g + 1) * 64, :]
            vt_ref[:, b * TQ:(b + 1) * TQ] = pltpu.bitcast(qv[D:2 * D].astype(bf16), u32)
            va = jnp.max(jnp.abs(qv[D:2 * D]).reshape(D // 8, 8, TQ), axis=0)
            vmax = va if b == 0 else jnp.maximum(vmax, va)
            qh = pltpu.bitcast(q_rows(0, b), bf16).astype(f32)
            for d in range(DH):
                qba_ref[b, d * 8:(d + 1) * 8, :] = jnp.broadcast_to(qh[d:d + 1, :], (8, TQ))

        misc_ref[VM, :] = vmax

        def do_pv(st, h, u, c, p):
            vv = pltpu.bitcast(vt_ref[pl.ds(aligned(h * 8, 8), 8), c * CK:(c + 1) * CK], bf16)
            st["acc"] = st["acc"] + lax.dot_general(
                vv, p, (((1,), (0,)), ((), ())), precision=lax.Precision.DEFAULT,
                preferred_element_type=f32)
            if c == NC - 1:
                ot_ref[u, pl.ds(aligned(h * DH, DH), DH), :] = st["acc"]
                l_ref[u, pl.ds(h, 1), :] = jnp.sum(st["l"], axis=0, keepdims=True)

        def carried(hprev):
            st = dict(acc=misc_ref[AC, :], l=misc_ref[LC, :])
            return {x: (st, hprev, t[0], t[1], pc_ref[i]) for i, (t, x) in enumerate(P.carry)}

        def head(h, qb_ref, kb_ref, kr_ref, hn, qbn_ref, kbn_ref, krn_ref):
            cpend = carried(jnp.maximum(h - 1, 0))
            fmask = zi_ref[0:8, :] != 0
            fmask4 = jnp.concatenate([fmask] * 4, axis=1)
            st, sv, pg, qhn, ptile, uidx = {}, {}, {}, {}, {}, {}

            def finish(u, blks, sx):
                p = jnp.exp2(sx)
                ps = [p[i * 8:(i + 1) * 8] for i in range(len(blks))] if len(blks) > 1 else [p]
                t = ps[0] + ps[1] if len(blks) == 2 else ps[0]
                st[u]["l"] = t if st[u]["l"] is None else st[u]["l"] + t
                for (c, b), pp in zip(blks, ps):
                    pg[u, c, b] = pp

            def run_segs(key, src):
                for (u2, kb, d0) in P.segpos.get(key, []):
                    if d0 == 0:
                        uidx[u2, kb] = u2 + zs_ref[kb]
                    qb = qb_ref[uidx[u2, kb], d0 * 8:(d0 + SEG) * 8, :]
                    kk = kb_ref[kb, d0 * 8:(d0 + SEG) * 8, :]
                    if src is not None:
                        kk = jnp.concatenate([lax.select(fmask, src, kk[0:8]), kk[8:]], axis=0)
                    pr = jnp.concatenate([kk] * 4, axis=1) * qb
                    for d in range(SEG):
                        t = pr[d * 8:(d + 1) * 8]
                        sv[u2, kb] = sv[u2, kb] + t if (u2, kb) in sv else t

            kro = roll_ko(hn)
            make_kr(krn_ref, hn)
            run_segs(-1, None)
            for (x0, x1) in P.pieces:
                u = P.stream[x0][0]
                if u not in st:
                    st[u] = dict(w=q_weights(h, u), l=None, acc=misc_ref[ZR, :])
                i0 = x0 - u * P.ng
                kk_ = pltpu.bitcast(kr_ref[i0 * 8:(i0 + x1 - x0) * 8, :], bf16)
                s = jnp.dot(kk_, st[u]["w"], preferred_element_type=f32)
                for x in range(x0, x1):
                    _, blk0, blk1 = P.stream[x]
                    r = (x - x0) * 16
                    for half in range(2):
                        if 2 * x + half in P.segpos:
                            run_segs(2 * x + half, s[r + 8 * half:r + 8 * half + 8, 0:128])
                    finish(u, (blk0, blk1), s[r:r + 16])
                    for (u3, d3) in P.qbpos.get(x, []):
                        if u3 not in qhn:
                            qhn[u3] = pltpu.bitcast(q_rows(hn, u3), bf16).astype(f32)
                        val = jnp.broadcast_to(qhn[u3][d3:d3 + 1, :], (8, TQ))
                        qbn_ref[u3, d3 * 8:(d3 + 1) * 8, :] = lax.select(fmask4, s[r:r + 8], val)
                    if x == KBX:
                        make_kb(kbn_ref, kro)
                    for c in sorted({blk0[0], blk1[0]}):
                        if x == P.last[u, c]:
                            bs = list(range(NV[c]))
                            while bs:
                                take, bs = bs[:2], bs[2:]
                                vals = [sv.pop((u, KB0[c] + b)) for b in take]
                                finish(u, [(c, b) for b in take],
                                       jnp.concatenate(vals, axis=0) if len(vals) > 1 else vals[0])
                            ptile[u, c] = jnp.concatenate(
                                [pg.pop((u, c, b)) for b in range(16)], axis=0)
                if x1 - 1 in cpend:
                    do_pv(*cpend.pop(x1 - 1))
                for t in P.pv_after.get(x1 - 1, []):
                    do_pv(st[t[0]], h, t[0], t[1], ptile.pop(t))
            misc_ref[AC, :] = st[NQ - 1]["acc"]
            misc_ref[LC, :] = st[NQ - 1]["l"]
            for i, (t, _) in enumerate(P.carry):
                pc_ref[i] = ptile.pop(t)

        def body(i, carry):
            @pl.when(i % 2 == 0)
            def _():
                head(i, qba_ref, kba_ref, kra_ref, i + 1, qbb_ref, kbb_ref, krb_ref)

            @pl.when(i % 2 == 1)
            def _():
                head(i, qbb_ref, kbb_ref, krb_ref, jnp.minimum(i + 1, H - 1),
                     qba_ref, kba_ref, kra_ref)
            return carry

        lax.fori_loop(0, H, body, 0)
        for item in carried(H - 1).values():
            do_pv(*item)
        ob_ref[...] = pltpu.bitcast(o_block(0, 0), u32)

        lall = l_ref[...].reshape(NQ * H, TQ)
        bad_l = jnp.where(jnp.logical_and(lall >= L_LO, lall <= L_HI), 0.0, 1.0)
        bad_v = jnp.where(misc_ref[VM, :] <= V_HI, 0.0, 1.0)
        bad = jnp.maximum(jnp.max(bad_l.reshape(NQ * H // 8, 8, TQ), axis=0), bad_v)

        @pl.when(jnp.max(bad) > 0.0)
        def _exact():
            rowgrp = lax.broadcasted_iota(i32, (64, TQ), 0) // (DH // 2)

            def fb(t, carry):
                u = t // H
                h = t % H
                q = qt_ref[u * 4 + h // 8]
                w = pltpu.bitcast(jnp.where(rowgrp == h % 8, q, jnp.zeros_like(q)), bf16)

                def scores(cb, m):
                    kk = pltpu.bitcast(
                        k_ref[h // 8, pl.ds(pl.multiple_of(cb * 256, 256), 256), :], bf16)
                    s = jnp.dot(kk, w, preferred_element_type=f32)
                    s_ref[pl.ds(pl.multiple_of(cb * 512, 512), 512), :] = s
                    return jnp.maximum(m, jnp.max(s.reshape(64, 8, TQ), axis=0))

                m = lax.fori_loop(0, S // 512, scores, jnp.full((8, TQ), -jnp.inf, f32))
                m = jnp.max(m, axis=0, keepdims=True)

                def pv(cb, la):
                    l, acc = la
                    off = pl.multiple_of(cb * 512, 512)
                    p = jnp.exp2(s_ref[pl.ds(off, 512), :] - m)
                    l = l + jnp.sum(p.reshape(64, 8, TQ), axis=0)
                    vv = pltpu.bitcast(
                        vt_ref[pl.ds(pl.multiple_of(h * 8, 8), 8), pl.ds(off, 512)], bf16)
                    acc = acc + jnp.dot(vv, p.astype(bf16), preferred_element_type=f32)
                    return l, acc

                l, acc = lax.fori_loop(
                    0, S // 512, pv, (jnp.zeros((8, TQ), f32), jnp.zeros((DH, TQ), f32)))
                ot_ref[u, pl.ds(pl.multiple_of(h * DH, DH), DH), :] = acc
                l_ref[u, pl.ds(h, 1), :] = jnp.sum(l, axis=0, keepdims=True)
                return carry

            lax.fori_loop(0, NQ * H, fb, 0)
            ob_ref[...] = pltpu.bitcast(o_block(0, 0), u32)

        for cp in late_copies():
            cp.wait()

    b1 = bias_ref[0:F].astype(f32)[None, :]
    b2 = bias_ref[2048:2048 + D].astype(f32)[None, :]

    def out_copy(j):
        return pltpu.make_async_copy(o_ref.at[j], o_hbm.at[pl.ds(aligned(j * TS, TS), TS), :],
                                     osem.at[j])

    hs, hns = [], []
    for i in range(NSUB):
        r0 = pl.multiple_of(step * TM + i * TS, TS)
        o = pltpu.bitcast(ob_ref[...], bf16) if i == 0 else o_block(step, i)
        attn = jnp.dot(o, wo_ref[...], preferred_element_type=f32)
        h = x_ref[pl.ds(r0, TS), :].astype(f32) + attn
        hs.append(h)
        hns.append(_layernorm(h).astype(bf16))
    for i in range(NSUB):
        a = jnp.dot(hns[i], w1_ref[...], preferred_element_type=f32) + b1
        a = jax.nn.gelu(a, approximate=True).astype(bf16)
        y = jnp.dot(a, w2_ref[...], preferred_element_type=f32) + b2
        o_ref[step * NSUB + i] = (hs[i] + y).astype(o_ref.dtype)
        out_copy(step * NSUB + i).start()
    ob_ref[...] = pltpu.bitcast(o_block(jnp.minimum(step + 1, NB - 1), 0), u32)

    @pl.when(step == NB - 1)
    def _():
        for j in range(NB * NSUB):
            out_copy(j).wait()


@jax.jit
def pallas_sequential_preLN__softmax_full_mha__dense_activation_gelu__prompt_kernel(
    A_x: jax.Array,
    A_wqkv: jax.Array,
    A_wo: jax.Array,
    B_x: jax.Array,
    B_w1: jax.Array,
    B_b1: jax.Array,
    B_w2: jax.Array,
    B_b2: jax.Array,
):
    del B_x
    x = A_x.reshape(S, D)
    hbm = pl.BlockSpec(memory_space=pl.ANY)
    tables = [
        pltpu.VMEM((NQ, DH * 8, TQ), f32),
        pltpu.VMEM((RPAD // 8, DH * 8, 128), f32),
        pltpu.VMEM((1024, 128), u32),
    ]

    out = pl.pallas_call(
        _kernel,
        grid=(NB,),
        in_specs=[hbm] * 7,
        out_specs=hbm,
        out_shape=jax.ShapeDtypeStruct((S, D), A_x.dtype),
        scratch_shapes=[
            pltpu.VMEM((S, D), bf16),
            pltpu.VMEM((D, D), bf16),
            pltpu.VMEM((D, D), bf16),
            pltpu.VMEM((D, D), bf16),
            pltpu.VMEM((D, D), bf16),
            pltpu.VMEM((D, F), bf16),
            pltpu.VMEM((F, D), bf16),
            pltpu.SemaphoreType.DMA((NX + 8,)),
            pltpu.VMEM((S // 2, D), u32),
            pltpu.VMEM((4, S // 2, 128), u32),
            pltpu.VMEM((4, S // 2, 128), u32),
            pltpu.VMEM((NQ * 4, 64, TQ), u32),
            pltpu.VMEM((D // 2, S), u32),
            pltpu.VMEM((4, RPAD, 128), f32),
        ] + tables + tables + [
            pltpu.VMEM((NCARRY, CK, TQ), f32),
            pltpu.VMEM((64, TQ), f32),
            pltpu.VMEM((128, 128), i32),
            pltpu.SMEM((NKB,), i32),
            pltpu.VMEM((NQ, D, TQ), f32),
            pltpu.VMEM((NQ, H, TQ), f32),
            pltpu.VMEM((TS // 2, D), u32),
            pltpu.VMEM((S, TQ), f32),
            pltpu.VMEM((32768,), bf16),
            pltpu.VMEM((S // TS, TS, D), bf16),
            pltpu.SemaphoreType.DMA((S // TS,)),
        ],
        compiler_params=pltpu.CompilerParams(
            dimension_semantics=("arbitrary",),
            vmem_limit_bytes=100 * 1024 * 1024,
        ),
    )(x, A_wqkv, A_wo, B_w1, B_w2, B_b1, B_b2)
    return out.reshape(1, S, D)
```

```python
import jax
import jax.numpy as jnp
from jax import lax
import jax.experimental.pallas as pl
import jax.experimental.pallas.tpu as pltpu

S = 2048
D = 512
H = 32
DH = 16
F = 1792
TQ = 512
NQ = S // TQ
CK = 128
NC = S // CK
TM = 512
NB = S // TM
NSUB = 2
TS = TM // NSUB
XCH = [(0, 256), (256, 256), (512, 512), (1024, 512), (1536, 512)]
NX = len(XCH)
EPS = 1e-5
QSCALE = (DH ** -0.5) * 1.4426950408889634

NV = [2 + c % 2 for c in range(NC)]
KB0 = [sum(NV[:c]) for c in range(NC + 1)]
MB0 = [16 * c - KB0[c] for c in range(NC + 1)]
NKB = KB0[NC]
RV = NKB * 8
RPAD = 384
SEG = 4
SHIFT = 2
LAGG = 8
KBX = 8
L_LO = 2.0 ** -10
L_HI = 2.0 ** 64
V_HI = 2.0 ** 60

f32 = jnp.float32
bf16 = jnp.bfloat16
i32 = jnp.int32
u32 = jnp.uint32


def _layernorm(x):
    m = jnp.mean(x, axis=-1, keepdims=True)
    xc = x - m
    v = jnp.mean(xc * xc, axis=-1, keepdims=True)
    return xc * lax.rsqrt(v + EPS)


class _Plan:
    def __init__(self):
        blocks = [(c, b) for c in range(NC) for b in range(15, NV[c] - 1, -1)]
        assert len(blocks) % 2 == 0
        self.ng = len(blocks) // 2
        self.stream = [(u, blocks[2 * i], blocks[2 * i + 1])
                       for u in range(NQ) for i in range(self.ng)]
        ns = self.ns = len(self.stream)
        self.last, self.lasth = {}, {}
        for x, (u, b0, b1) in enumerate(self.stream):
            for half, (c, b) in enumerate((b0, b1)):
                self.last[u, c] = x
                self.lasth[u, c] = 2 * x + half
        tiles = [(u, c) for u in range(NQ) for c in range(NC)]
        self.pv_after, self.carry = {}, []
        for t in tiles:
            x = self.last[t] + LAGG
            if x <= ns - 1:
                self.pv_after.setdefault(x, []).append(t)
            else:
                self.carry.append((t, x - ns))
        assert all(t[0] == NQ - 1 for t, _ in self.carry)
        cuts = set(self.pv_after) | {x for _, x in self.carry} | {
            x for x in range(ns) if x == ns - 1 or self.stream[x + 1][0] != self.stream[x][0]}
        self.pieces, x0 = [], 0
        for x in range(ns):
            if x in cuts:
                self.pieces.append((x0, x + 1))
                x0 = x + 1
        segs = [(t, kb, d0) for t in tiles
                for kb in range(KB0[t[1]], KB0[t[1] + 1])
                for d0 in range(0, DH, SEG)]
        slots = []
        cx = {x for _, x in self.carry}
        for (x0, x1) in self.pieces:
            slots += list(range(2 * x0, 2 * x1))
            if x1 - 1 in self.pv_after or x1 - 1 in cx:
                slots += [('pv', x1 - 1, 0), ('pv', x1 - 1, 1)]
        sidx = {k: i for i, k in enumerate(slots)}
        self.segpos = {}
        for i, (t, kb, d0) in enumerate(segs):
            pos = min((i * len(slots)) // len(segs) - SHIFT, sidx[self.lasth[t]])
            self.segpos.setdefault(slots[pos] if pos >= 0 else -1, []).append((t[0], kb, d0))
        items = [(u, d) for u in range(NQ) for d in range(DH)]
        self.qbpos = {}
        for i, it in enumerate(items):
            self.qbpos.setdefault((i * (ns - 8)) // len(items), []).append(it)


PLAN = _Plan()
NCARRY = len(PLAN.carry)


def _kernel(x_hbm, wqkv_hbm, wo_hbm, w1_hbm, w2_hbm, b1_hbm, b2_hbm, o_hbm,
            x_ref, wq_ref, wk_ref, wv_ref, wo_ref, w1_ref, w2_ref, sem,
            xn_ref, k_ref, ks_ref, qt_ref, vt_ref, ko_ref,
            qba_ref, kba_ref, kra_ref, qbb_ref, kbb_ref, krb_ref,
            pc_ref, misc_ref, zi_ref, zs_ref, ot_ref, l_ref, ob_ref, s_ref, bias_ref, o_ref, osem):
    step = pl.program_id(0)
    P = PLAN
    AC, ZR, VM, LC = slice(0, 16), slice(16, 32), slice(32, 40), slice(48, 56)
    KL = slice(56, 64)

    def x_copy(i):
        r0, n = XCH[i]
        return pltpu.make_async_copy(x_hbm.at[pl.ds(r0, n), :], x_ref.at[pl.ds(r0, n), :],
                                     sem.at[i])

    def w_copy(i):
        dst = (wq_ref, wk_ref, wv_ref)[i]
        return pltpu.make_async_copy(wqkv_hbm.at[:, pl.ds(i * D, D)], dst, sem.at[NX + i])

    def late_copies():
        return (pltpu.make_async_copy(wo_hbm, wo_ref, sem.at[NX + 3]),
                pltpu.make_async_copy(w1_hbm, w1_ref, sem.at[NX + 4]),
                pltpu.make_async_copy(w2_hbm, w2_ref, sem.at[NX + 5]),
                pltpu.make_async_copy(b1_hbm, bias_ref.at[pl.ds(0, F)], sem.at[NX + 6]),
                pltpu.make_async_copy(b2_hbm, bias_ref.at[pl.ds(2048, D)], sem.at[NX + 7]))

    def aligned(i, m):
        return i if isinstance(i, int) else pl.multiple_of(i, m)

    def head_shift(h):
        return (128 - (h % 8) * DH) % 128

    def q_rows(h, u):
        return qt_ref[u * 4 + h // 8, pl.ds(aligned((h % 8) * 8, 8), 8), :]

    def q_weights(h, u):
        q16 = pltpu.bitcast(q_rows(h, u), bf16)
        return jnp.concatenate([q16, jnp.zeros((128 - DH, TQ), bf16)], axis=0)

    def roll_ko(h):
        return pltpu.roll(ko_ref[h // 8, 0:RV, :], head_shift(h), 1)

    def make_kb(kb_ref, kro):
        for d in range(DH):
            kb_ref[0:NKB, d * 8:(d + 1) * 8, :] = jnp.broadcast_to(
                kro[:, d:d + 1], (RV, 128)).reshape(NKB, 8, 128)

    def make_kr(kr_ref, h):
        kr_ref[0:P.ng * 8, :] = pltpu.roll(ks_ref[h // 8, 0:P.ng * 8, :], head_shift(h), 1)

    def o_block(u, i):
        linv = 1.0 / l_ref[u, :, i * TS:(i + 1) * TS]
        o = jnp.concatenate(
            [ot_ref[u, h * DH:(h + 1) * DH, i * TS:(i + 1) * TS] * linv[h:h + 1, :]
             for h in range(H)], axis=0)
        return o.T.astype(bf16)

    @pl.when(step == 0)
    def _attention():
        x_copy(0).start()
        w_copy(1).start()
        for i in range(1, NX):
            x_copy(i).start()
        w_copy(0).start()
        w_copy(2).start()

        misc_ref[0:32, :] = jnp.zeros((32, TQ), f32)
        misc_ref[LC, :] = jnp.ones((8, TQ), f32)
        zi_ref[0:8, :] = jnp.zeros((8, 128), i32)
        pc_ref[...] = jnp.zeros_like(pc_ref)
        for i in range(NKB):
            zs_ref[i] = 0

        def ln_chunk(r0, n, pace=None):
            x = x_ref[r0:r0 + n, :].astype(f32)
            if pace is not None:
                fm = zi_ref[0:8, :] != 0
                m, nj = pace.shape[0] // 8, n // 8
                parts = []
                for j in range(nj):
                    pr, pc = (j * 3 * m) // nj % m, (j * 3) // nj
                    parts.append(jnp.where(fm, pace[pr * 8:pr * 8 + 8, pc * 128:pc * 128 + 128],
                                           x[j * 8:(j + 1) * 8, 0:128]))
                x0 = jnp.concatenate(parts, axis=0)
                x = jnp.concatenate([x0, x[:, 128:]], axis=1)
            xn_ref[r0 // 2:(r0 + n) // 2, :] = pltpu.bitcast(_layernorm(x).astype(bf16), u32)

        def k_chunk(r0, n):
            xn = pltpu.bitcast(xn_ref[r0 // 2:(r0 + n) // 2, :], bf16)
            kf = jnp.dot(xn, wk_ref[...], preferred_element_type=f32)
            kb16 = kf.astype(bf16)
            kpk = pltpu.bitcast(kb16, u32)
            c0, c1 = r0 // CK, (r0 + n) // CK
            blks = [kf[(c - c0) * CK + b * 8:(c - c0) * CK + b * 8 + 8]
                    for c in range(c0, c1) for b in range(15, NV[c] - 1, -1)]
            if MB0[c0] % 2:
                blks = [misc_ref[KL, :]] + blks
            if MB0[c1] % 2:
                misc_ref[KL, :] = blks.pop()
            kspk = pltpu.bitcast(jnp.concatenate(blks, axis=0).astype(bf16), u32)
            kof = jnp.concatenate(
                [kf[(c - c0) * CK:(c - c0) * CK + 8 * NV[c]] for c in range(c0, c1)], axis=0)
            kof = kof.astype(bf16).astype(f32)
            for g in range(4):
                k_ref[g, r0 // 2:(r0 + n) // 2, :] = kpk[:, g * 128:(g + 1) * 128]
                ks_ref[g, MB0[c0] // 2 * 8:MB0[c1] // 2 * 8, :] = kspk[:, g * 128:(g + 1) * 128]
                ko_ref[g, KB0[c0] * 8:KB0[c1] * 8, :] = kof[:, g * 128:(g + 1) * 128]
            return kf

        x_copy(0).wait()
        ln_chunk(0, 256)
        w_copy(1).wait()
        x_copy(1).wait()
        ln_chunk(256, 256, k_chunk(0, 256))
        x_copy(2).wait()
        ln_chunk(512, 512, k_chunk(256, 256))
        x_copy(3).wait()
        kf = k_chunk(512, 512)
        ln_chunk(1024, 256)
        ln_chunk(1280, 256, kf)
        k_chunk(1024, 256)
        x_copy(4).wait()
        w_copy(0).wait()
        w_copy(2).wait()
        for cp in late_copies():
            cp.start()
        k_chunk(1280, 256)
        ln_chunk(1536, 512)
        k_chunk(1536, 512)
        wqv_t = jnp.concatenate(
            [wq_ref[...].astype(f32).T.astype(bf16), wv_ref[...].astype(f32).T.astype(bf16)],
            axis=0)
        nt = (((1,), (1,)), ((), ()))
        make_kb(kba_ref, roll_ko(0))
        make_kr(kra_ref, 0)
        for b in range(NQ):
            xn = pltpu.bitcast(xn_ref[b * TQ // 2:(b + 1) * TQ // 2, :], bf16)
            qv = lax.dot_general(wqv_t, xn, nt, preferred_element_type=f32)
            qt = pltpu.bitcast((qv[0:D] * QSCALE).astype(bf16), u32)
            for g in range(4):
                qt_ref[b * 4 + g] = qt[g * 64:(g + 1) * 64, :]
            vt_ref[:, b * TQ:(b + 1) * TQ] = pltpu.bitcast(qv[D:2 * D].astype(bf16), u32)
            va = jnp.max(jnp.abs(qv[D:2 * D]).reshape(D // 8, 8, TQ), axis=0)
            vmax = va if b == 0 else jnp.maximum(vmax, va)
            qh = pltpu.bitcast(q_rows(0, b), bf16).astype(f32)
            for d in range(DH):
                qba_ref[b, d * 8:(d + 1) * 8, :] = jnp.broadcast_to(qh[d:d + 1, :], (8, TQ))

        misc_ref[VM, :] = vmax

        def do_pv(st, h, u, c, p):
            vv = pltpu.bitcast(vt_ref[pl.ds(aligned(h * 8, 8), 8), c * CK:(c + 1) * CK], bf16)
            st["acc"] = st["acc"] + lax.dot_general(
                vv, p, (((1,), (0,)), ((), ())), precision=lax.Precision.DEFAULT,
                preferred_element_type=f32)
            res = st["acc"]
            if c == NC - 1:
                ot_ref[u, pl.ds(aligned(h * DH, DH), DH), :] = st["acc"]
                l_ref[u, pl.ds(h, 1), :] = jnp.sum(st["l"], axis=0, keepdims=True)
            return res

        def carried(hprev):
            st = dict(acc=misc_ref[AC, :], l=misc_ref[LC, :])
            out = {}
            for i, (t, x) in enumerate(P.carry):
                p = pc_ref[i]
                if i == NCARRY - 1:
                    p = jnp.exp2(p)
                    for j in range(CK // 16 - 1, -1, -1):
                        st["l"] = st["l"] + (p[j * 16:j * 16 + 8] + p[j * 16 + 8:j * 16 + 16])
                out[x] = (st, hprev, t[0], t[1], p)
            return out

        def head(h, qb_ref, kb_ref, kr_ref, hn, qbn_ref, kbn_ref, krn_ref):
            cpend = carried(jnp.maximum(h - 1, 0))
            fmask = zi_ref[0:8, :] != 0
            fmask4 = jnp.concatenate([fmask] * 4, axis=1)
            st, sv, pg, qhn, ptile, uidx = {}, {}, {}, {}, {}, {}

            ctiles = {P.carry[-1][0]}

            def finish(u, blks, sx):
                xs = [sx[i * 8:(i + 1) * 8] for i in range(len(blks))] if len(blks) > 1 else [sx]
                live = [i for i, (c, b) in enumerate(blks) if (u, c) not in ctiles]
                for i, (c, b) in enumerate(blks):
                    pg[u, c, b] = jnp.exp2(xs[i]) if i in live else xs[i]
                if live:
                    ps = [pg[(u,) + blks[i]] for i in live]
                    t = ps[0] + ps[1] if len(ps) == 2 else ps[0]
                    st[u]["l"] = t if st[u]["l"] is None else st[u]["l"] + t

            def run_segs(key, src):
                for (u2, kb, d0) in P.segpos.get(key, []):
                    if d0 == 0:
                        uidx[u2, kb] = u2 + zs_ref[kb]
                    qb = qb_ref[uidx[u2, kb], d0 * 8:(d0 + SEG) * 8, :]
                    kk = kb_ref[kb, d0 * 8:(d0 + SEG) * 8, :]
                    if src is not None:
                        kk = jnp.concatenate([lax.select(fmask, src, kk[0:8]), kk[8:]], axis=0)
                    pr = jnp.concatenate([kk] * 4, axis=1) * qb
                    for d in range(SEG):
                        t = pr[d * 8:(d + 1) * 8]
                        sv[u2, kb] = sv[u2, kb] + t if (u2, kb) in sv else t

            kro = roll_ko(hn)
            make_kr(krn_ref, hn)
            run_segs(-1, None)
            for (x0, x1) in P.pieces:
                u = P.stream[x0][0]
                if u not in st:
                    st[u] = dict(w=q_weights(h, u), l=None, acc=misc_ref[ZR, :])
                i0 = x0 - u * P.ng
                kk_ = pltpu.bitcast(kr_ref[i0 * 8:(i0 + x1 - x0) * 8, :], bf16)
                s = jnp.dot(kk_, st[u]["w"], preferred_element_type=f32)
                for x in range(x0, x1):
                    _, blk0, blk1 = P.stream[x]
                    r = (x - x0) * 16
                    for half in range(2):
                        if 2 * x + half in P.segpos:
                            run_segs(2 * x + half, s[r + 8 * half:r + 8 * half + 8, 0:128])
                    finish(u, (blk0, blk1), s[r:r + 16])
                    for (u3, d3) in P.qbpos.get(x, []):
                        if u3 not in qhn:
                            qhn[u3] = pltpu.bitcast(q_rows(hn, u3), bf16).astype(f32)
                        val = jnp.broadcast_to(qhn[u3][d3:d3 + 1, :], (8, TQ))
                        qbn_ref[u3, d3 * 8:(d3 + 1) * 8, :] = lax.select(fmask4, s[r:r + 8], val)
                    if x == KBX:
                        make_kb(kbn_ref, kro)
                    for c in sorted({blk0[0], blk1[0]}):
                        if x == P.last[u, c]:
                            bs = list(range(NV[c]))
                            while bs:
                                take, bs = bs[:2], bs[2:]
                                vals = [sv.pop((u, KB0[c] + b)) for b in take]
                                finish(u, [(c, b) for b in take],
                                       jnp.concatenate(vals, axis=0) if len(vals) > 1 else vals[0])
                            ptile[u, c] = jnp.concatenate(
                                [pg.pop((u, c, b)) for b in range(16)], axis=0)
                if x1 - 1 in cpend:
                    res = do_pv(*cpend.pop(x1 - 1))
                for t in P.pv_after.get(x1 - 1, []):
                    res = do_pv(st[t[0]], h, t[0], t[1], ptile.pop(t))
                for half in range(2):
                    if ('pv', x1 - 1, half) in P.segpos:
                        run_segs(('pv', x1 - 1, half), res[8 * half:8 * half + 8, 0:128])
            misc_ref[AC, :] = st[NQ - 1]["acc"]
            misc_ref[LC, :] = st[NQ - 1]["l"]
            for i, (t, _) in enumerate(P.carry):
                pc_ref[i] = ptile.pop(t)

        def body(i, carry):
            @pl.when(i % 2 == 0)
            def _():
                head(i, qba_ref, kba_ref, kra_ref, i + 1, qbb_ref, kbb_ref, krb_ref)

            @pl.when(i % 2 == 1)
            def _():
                head(i, qbb_ref, kbb_ref, krb_ref, jnp.minimum(i + 1, H - 1),
                     qba_ref, kba_ref, kra_ref)
            return carry

        lax.fori_loop(0, H, body, 0)
        for item in carried(H - 1).values():
            do_pv(*item)
        ob_ref[...] = pltpu.bitcast(o_block(0, 0), u32)

        lall = l_ref[...].reshape(NQ * H, TQ)
        bad_l = jnp.where(jnp.logical_and(lall >= L_LO, lall <= L_HI), 0.0, 1.0)
        bad_v = jnp.where(misc_ref[VM, :] <= V_HI, 0.0, 1.0)
        bad = jnp.maximum(jnp.max(bad_l.reshape(NQ * H // 8, 8, TQ), axis=0), bad_v)

        @pl.when(jnp.max(bad) > 0.0)
        def _exact():
            rowgrp = lax.broadcasted_iota(i32, (64, TQ), 0) // (DH // 2)

            def fb(t, carry):
                u = t // H
                h = t % H
                q = qt_ref[u * 4 + h // 8]
                w = pltpu.bitcast(jnp.where(rowgrp == h % 8, q, jnp.zeros_like(q)), bf16)

                def scores(cb, m):
                    kk = pltpu.bitcast(
                        k_ref[h // 8, pl.ds(pl.multiple_of(cb * 256, 256), 256), :], bf16)
                    s = jnp.dot(kk, w, preferred_element_type=f32)
                    s_ref[pl.ds(pl.multiple_of(cb * 512, 512), 512), :] = s
                    return jnp.maximum(m, jnp.max(s.reshape(64, 8, TQ), axis=0))

                m = lax.fori_loop(0, S // 512, scores, jnp.full((8, TQ), -jnp.inf, f32))
                m = jnp.max(m, axis=0, keepdims=True)

                def pv(cb, la):
                    l, acc = la
                    off = pl.multiple_of(cb * 512, 512)
                    p = jnp.exp2(s_ref[pl.ds(off, 512), :] - m)
                    l = l + jnp.sum(p.reshape(64, 8, TQ), axis=0)
                    vv = pltpu.bitcast(
                        vt_ref[pl.ds(pl.multiple_of(h * 8, 8), 8), pl.ds(off, 512)], bf16)
                    acc = acc + jnp.dot(vv, p.astype(bf16), preferred_element_type=f32)
                    return l, acc

                l, acc = lax.fori_loop(
                    0, S // 512, pv, (jnp.zeros((8, TQ), f32), jnp.zeros((DH, TQ), f32)))
                ot_ref[u, pl.ds(pl.multiple_of(h * DH, DH), DH), :] = acc
                l_ref[u, pl.ds(h, 1), :] = jnp.sum(l, axis=0, keepdims=True)
                return carry

            lax.fori_loop(0, NQ * H, fb, 0)
            ob_ref[...] = pltpu.bitcast(o_block(0, 0), u32)

        for cp in late_copies():
            cp.wait()

    b1 = bias_ref[0:F].astype(f32)[None, :]
    b2 = bias_ref[2048:2048 + D].astype(f32)[None, :]

    def out_copy(j):
        return pltpu.make_async_copy(o_ref.at[j], o_hbm.at[pl.ds(aligned(j * TS, TS), TS), :],
                                     osem.at[j])

    hs, hns = [], []
    for i in range(NSUB):
        r0 = pl.multiple_of(step * TM + i * TS, TS)
        o = pltpu.bitcast(ob_ref[...], bf16) if i == 0 else o_block(step, i)
        attn = jnp.dot(o, wo_ref[...], preferred_element_type=f32)
        h = x_ref[pl.ds(r0, TS), :].astype(f32) + attn
        hs.append(h)
        hns.append(_layernorm(h).astype(bf16))
    for i in range(NSUB):
        a = jnp.dot(hns[i], w1_ref[...], preferred_element_type=f32) + b1
        a = jax.nn.gelu(a, approximate=True).astype(bf16)
        y = jnp.dot(a, w2_ref[...], preferred_element_type=f32) + b2
        o_ref[step * NSUB + i] = (hs[i] + y).astype(o_ref.dtype)
        out_copy(step * NSUB + i).start()
    ob_ref[...] = pltpu.bitcast(o_block(jnp.minimum(step + 1, NB - 1), 0), u32)

    @pl.when(step == NB - 1)
    def _():
        for j in range(NB * NSUB):
            out_copy(j).wait()


@jax.jit
def pallas_sequential_preLN__softmax_full_mha__dense_activation_gelu__prompt_kernel(
    A_x: jax.Array,
    A_wqkv: jax.Array,
    A_wo: jax.Array,
    B_x: jax.Array,
    B_w1: jax.Array,
    B_b1: jax.Array,
    B_w2: jax.Array,
    B_b2: jax.Array,
):
    del B_x
    x = A_x.reshape(S, D)
    hbm = pl.BlockSpec(memory_space=pl.ANY)
    tables = [
        pltpu.VMEM((NQ, DH * 8, TQ), f32),
        pltpu.VMEM((RPAD // 8, DH * 8, 128), f32),
        pltpu.VMEM((1024, 128), u32),
    ]

    out = pl.pallas_call(
        _kernel,
        grid=(NB,),
        in_specs=[hbm] * 7,
        out_specs=hbm,
        out_shape=jax.ShapeDtypeStruct((S, D), A_x.dtype),
        scratch_shapes=[
            pltpu.VMEM((S, D), bf16),
            pltpu.VMEM((D, D), bf16),
            pltpu.VMEM((D, D), bf16),
            pltpu.VMEM((D, D), bf16),
            pltpu.VMEM((D, D), bf16),
            pltpu.VMEM((D, F), bf16),
            pltpu.VMEM((F, D), bf16),
            pltpu.SemaphoreType.DMA((NX + 8,)),
            pltpu.VMEM((S // 2, D), u32),
            pltpu.VMEM((4, S // 2, 128), u32),
            pltpu.VMEM((4, S // 2, 128), u32),
            pltpu.VMEM((NQ * 4, 64, TQ), u32),
            pltpu.VMEM((D // 2, S), u32),
            pltpu.VMEM((4, RPAD, 128), f32),
        ] + tables + tables + [
            pltpu.VMEM((NCARRY, CK, TQ), f32),
            pltpu.VMEM((64, TQ), f32),
            pltpu.VMEM((128, 128), i32),
            pltpu.SMEM((NKB,), i32),
            pltpu.VMEM((NQ, D, TQ), f32),
            pltpu.VMEM((NQ, H, TQ), f32),
            pltpu.VMEM((TS // 2, D), u32),
            pltpu.VMEM((S, TQ), f32),
            pltpu.VMEM((32768,), bf16),
            pltpu.VMEM((S // TS, TS, D), bf16),
            pltpu.SemaphoreType.DMA((S // TS,)),
        ],
        compiler_params=pltpu.CompilerParams(
            dimension_semantics=("arbitrary",),
            vmem_limit_bytes=100 * 1024 * 1024,
        ),
    )(x, A_wqkv, A_wo, B_w1, B_w2, B_b1, B_b2)
    return out.reshape(1, S, D)
```

```python
import jax
import jax.numpy as jnp
from jax import lax
import jax.experimental.pallas as pl
import jax.experimental.pallas.tpu as pltpu

S = 2048
D = 512
H = 32
DH = 16
F = 1792
TQ = 512
NQ = S // TQ
CK = 128
NC = S // CK
TM = 512
NB = S // TM
NSUB = 2
TS = TM // NSUB
XCH = [(0, 256), (256, 256), (512, 512), (1024, 512), (1536, 512)]
NX = len(XCH)
EPS = 1e-5
QSCALE = (DH ** -0.5) * 1.4426950408889634

NV = [2 + c % 2 for c in range(NC)]
KB0 = [sum(NV[:c]) for c in range(NC + 1)]
MB0 = [16 * c - KB0[c] for c in range(NC + 1)]
NKB = KB0[NC]
RV = NKB * 8
RPAD = 384
SEG = 4
SHIFT = 2
LAGG = 8
KBX = 8
L_LO = 2.0 ** -10
L_HI = 2.0 ** 64
V_HI = 2.0 ** 60

f32 = jnp.float32
bf16 = jnp.bfloat16
i32 = jnp.int32
u32 = jnp.uint32


def _layernorm(x):
    m = jnp.mean(x, axis=-1, keepdims=True)
    xc = x - m
    v = jnp.mean(xc * xc, axis=-1, keepdims=True)
    return xc * lax.rsqrt(v + EPS)


class _Plan:
    def __init__(self):
        blocks = [(c, b) for c in range(NC) for b in range(15, NV[c] - 1, -1)]
        assert len(blocks) % 2 == 0
        self.ng = len(blocks) // 2
        self.stream = [(u, blocks[2 * i], blocks[2 * i + 1])
                       for u in range(NQ) for i in range(self.ng)]
        ns = self.ns = len(self.stream)
        self.last, self.lasth = {}, {}
        for x, (u, b0, b1) in enumerate(self.stream):
            for half, (c, b) in enumerate((b0, b1)):
                self.last[u, c] = x
                self.lasth[u, c] = 2 * x + half
        tiles = [(u, c) for u in range(NQ) for c in range(NC)]
        self.pv_after, self.carry = {}, []
        for t in tiles:
            x = self.last[t] + LAGG
            if x <= ns - 1:
                self.pv_after.setdefault(x, []).append(t)
            else:
                self.carry.append((t, x - ns))
        assert all(t[0] == NQ - 1 for t, _ in self.carry)
        cuts = set(self.pv_after) | {x for _, x in self.carry} | {
            x for x in range(ns) if x == ns - 1 or self.stream[x + 1][0] != self.stream[x][0]}
        self.pieces, x0 = [], 0
        for x in range(ns):
            if x in cuts:
                self.pieces.append((x0, x + 1))
                x0 = x + 1
        segs = [(t, kb, d0) for t in tiles
                for kb in range(KB0[t[1]], KB0[t[1] + 1])
                for d0 in range(0, DH, SEG)]
        slots = []
        cx = {x for _, x in self.carry}
        for (x0, x1) in self.pieces:
            slots += list(range(2 * x0, 2 * x1))
            if x1 - 1 in self.pv_after or x1 - 1 in cx:
                slots += [('pv', x1 - 1, 0), ('pv', x1 - 1, 1)]
        sidx = {k: i for i, k in enumerate(slots)}
        self.segpos = {}
        for i, (t, kb, d0) in enumerate(segs):
            pos = min((i * len(slots)) // len(segs) - SHIFT, sidx[self.lasth[t]])
            self.segpos.setdefault(slots[pos] if pos >= 0 else -1, []).append((t[0], kb, d0))
        items = [(u, d) for u in range(NQ) for d in range(DH)]
        self.qbpos = {}
        for i, it in enumerate(items):
            self.qbpos.setdefault((i * (ns - 8)) // len(items), []).append(it)


PLAN = _Plan()
NCARRY = len(PLAN.carry)


def _kernel(x_hbm, wqkv_hbm, wo_hbm, w1_hbm, w2_hbm, b1_hbm, b2_hbm, o_hbm,
            x_ref, wq_ref, wk_ref, wv_ref, wo_ref, w1_ref, w2_ref, sem,
            xn_ref, k_ref, ks_ref, qt_ref, vt_ref, ko_ref,
            qba_ref, kba_ref, kra_ref, qbb_ref, kbb_ref, krb_ref,
            pc_ref, misc_ref, zi_ref, zs_ref, ot_ref, l_ref, ob_ref, s_ref, bias_ref, o_ref, osem):
    step = pl.program_id(0)
    P = PLAN
    AC, ZR, VM, LC = slice(0, 16), slice(16, 32), slice(32, 40), slice(48, 56)
    KL = slice(56, 64)

    def x_copy(i):
        r0, n = XCH[i]
        return pltpu.make_async_copy(x_hbm.at[pl.ds(r0, n), :], x_ref.at[pl.ds(r0, n), :],
                                     sem.at[i])

    def w_copy(i):
        dst = (wq_ref, wk_ref, wv_ref)[i]
        return pltpu.make_async_copy(wqkv_hbm.at[:, pl.ds(i * D, D)], dst, sem.at[NX + i])

    def late_copies():
        return (pltpu.make_async_copy(wo_hbm, wo_ref, sem.at[NX + 3]),
                pltpu.make_async_copy(w1_hbm, w1_ref, sem.at[NX + 4]),
                pltpu.make_async_copy(w2_hbm, w2_ref, sem.at[NX + 5]),
                pltpu.make_async_copy(b1_hbm, bias_ref.at[pl.ds(0, F)], sem.at[NX + 6]),
                pltpu.make_async_copy(b2_hbm, bias_ref.at[pl.ds(2048, D)], sem.at[NX + 7]))

    def aligned(i, m):
        return i if isinstance(i, int) else pl.multiple_of(i, m)

    def head_shift(h):
        return (128 - (h % 8) * DH) % 128

    def q_rows(h, u):
        return qt_ref[u * 4 + h // 8, pl.ds(aligned((h % 8) * 8, 8), 8), :]

    def q_weights(kr_ref, u):
        r0 = (P.ng + 4 * u) * 8
        q8 = jnp.concatenate([kr_ref[r0 + t * 8:r0 + (t + 1) * 8, :] for t in range(4)], axis=1)
        return jnp.concatenate(
            [pltpu.bitcast(q8, bf16), jnp.zeros((128 - DH, TQ), bf16)], axis=0)

    def make_wq(kr_ref, q8, u):
        r0 = (P.ng + 4 * u) * 8
        for t in range(4):
            kr_ref[r0 + t * 8:r0 + (t + 1) * 8, :] = q8[:, t * 128:(t + 1) * 128]

    def roll_ko(h):
        return pltpu.roll(ko_ref[h // 8, 0:RV, :], head_shift(h), 1)

    def make_kb(kb_ref, kro):
        for d in range(DH):
            kb_ref[0:NKB, d * 8:(d + 1) * 8, :] = jnp.broadcast_to(
                kro[:, d:d + 1], (RV, 128)).reshape(NKB, 8, 128)

    def make_kr(kr_ref, h):
        kr_ref[0:P.ng * 8, :] = pltpu.roll(ks_ref[h // 8, 0:P.ng * 8, :], head_shift(h), 1)

    def o_block(u, i):
        linv = 1.0 / l_ref[u, :, i * TS:(i + 1) * TS]
        o = jnp.concatenate(
            [ot_ref[u, h * DH:(h + 1) * DH, i * TS:(i + 1) * TS] * linv[h:h + 1, :]
             for h in range(H)], axis=0)
        return o.T.astype(bf16)

    @pl.when(step == 0)
    def _attention():
        x_copy(0).start()
        w_copy(1).start()
        for i in range(1, NX):
            x_copy(i).start()
        w_copy(0).start()
        w_copy(2).start()

        misc_ref[0:32, :] = jnp.zeros((32, TQ), f32)
        misc_ref[LC, :] = jnp.ones((8, TQ), f32)
        zi_ref[0:8, :] = jnp.zeros((8, 128), i32)
        pc_ref[...] = jnp.zeros_like(pc_ref)
        for i in range(NKB):
            zs_ref[i] = 0

        def ln_chunk(r0, n, pace=None):
            x = x_ref[r0:r0 + n, :].astype(f32)
            if pace is not None:
                fm = zi_ref[0:8, :] != 0
                m, nj = pace.shape[0] // 8, n // 8
                parts = []
                for j in range(nj):
                    pr, pc = (j * 3 * m) // nj % m, (j * 3) // nj
                    parts.append(jnp.where(fm, pace[pr * 8:pr * 8 + 8, pc * 128:pc * 128 + 128],
                                           x[j * 8:(j + 1) * 8, 0:128]))
                x0 = jnp.concatenate(parts, axis=0)
                x = jnp.concatenate([x0, x[:, 128:]], axis=1)
            xn_ref[r0 // 2:(r0 + n) // 2, :] = pltpu.bitcast(_layernorm(x).astype(bf16), u32)

        def k_chunk(r0, n):
            xn = pltpu.bitcast(xn_ref[r0 // 2:(r0 + n) // 2, :], bf16)
            kf = jnp.dot(xn, wk_ref[...], preferred_element_type=f32)
            kb16 = kf.astype(bf16)
            kpk = pltpu.bitcast(kb16, u32)
            c0, c1 = r0 // CK, (r0 + n) // CK
            blks = [kf[(c - c0) * CK + b * 8:(c - c0) * CK + b * 8 + 8]
                    for c in range(c0, c1) for b in range(15, NV[c] - 1, -1)]
            if MB0[c0] % 2:
                blks = [misc_ref[KL, :]] + blks
            if MB0[c1] % 2:
                misc_ref[KL, :] = blks.pop()
            kspk = pltpu.bitcast(jnp.concatenate(blks, axis=0).astype(bf16), u32)
            kof = jnp.concatenate(
                [kf[(c - c0) * CK:(c - c0) * CK + 8 * NV[c]] for c in range(c0, c1)], axis=0)
            kof = kof.astype(bf16).astype(f32)
            for g in range(4):
                k_ref[g, r0 // 2:(r0 + n) // 2, :] = kpk[:, g * 128:(g + 1) * 128]
                ks_ref[g, MB0[c0] // 2 * 8:MB0[c1] // 2 * 8, :] = kspk[:, g * 128:(g + 1) * 128]
                ko_ref[g, KB0[c0] * 8:KB0[c1] * 8, :] = kof[:, g * 128:(g + 1) * 128]
            return kf

        x_copy(0).wait()
        ln_chunk(0, 256)
        w_copy(1).wait()
        x_copy(1).wait()
        ln_chunk(256, 256, k_chunk(0, 256))
        x_copy(2).wait()
        ln_chunk(512, 512, k_chunk(256, 256))
        x_copy(3).wait()
        kf = k_chunk(512, 512)
        ln_chunk(1024, 256)
        ln_chunk(1280, 256, kf)
        k_chunk(1024, 256)
        x_copy(4).wait()
        w_copy(0).wait()
        w_copy(2).wait()
        for cp in late_copies():
            cp.start()
        k_chunk(1280, 256)
        ln_chunk(1536, 512)
        k_chunk(1536, 512)
        wqv_t = jnp.concatenate(
            [wq_ref[...].astype(f32).T.astype(bf16), wv_ref[...].astype(f32).T.astype(bf16)],
            axis=0)
        nt = (((1,), (1,)), ((), ()))
        make_kb(kba_ref, roll_ko(0))
        make_kr(kra_ref, 0)
        for b in range(NQ):
            xn = pltpu.bitcast(xn_ref[b * TQ // 2:(b + 1) * TQ // 2, :], bf16)
            qv = lax.dot_general(wqv_t, xn, nt, preferred_element_type=f32)
            qt = pltpu.bitcast((qv[0:D] * QSCALE).astype(bf16), u32)
            for g in range(4):
                qt_ref[b * 4 + g] = qt[g * 64:(g + 1) * 64, :]
            vt_ref[:, b * TQ:(b + 1) * TQ] = pltpu.bitcast(qv[D:2 * D].astype(bf16), u32)
            va = jnp.max(jnp.abs(qv[D:2 * D]).reshape(D // 8, 8, TQ), axis=0)
            vmax = va if b == 0 else jnp.maximum(vmax, va)
            make_wq(kra_ref, q_rows(0, b), b)
            qh = pltpu.bitcast(q_rows(0, b), bf16).astype(f32)
            for d in range(DH):
                qba_ref[b, d * 8:(d + 1) * 8, :] = jnp.broadcast_to(qh[d:d + 1, :], (8, TQ))

        misc_ref[VM, :] = vmax

        def do_pv(st, h, u, c, p):
            vv = pltpu.bitcast(vt_ref[pl.ds(aligned(h * 8, 8), 8), c * CK:(c + 1) * CK], bf16)
            st["acc"] = st["acc"] + lax.dot_general(
                vv, p, (((1,), (0,)), ((), ())), precision=lax.Precision.DEFAULT,
                preferred_element_type=f32)
            res = st["acc"]
            if c == NC - 1:
                ot_ref[u, pl.ds(aligned(h * DH, DH), DH), :] = st["acc"]
                l_ref[u, pl.ds(h, 1), :] = jnp.sum(st["l"], axis=0, keepdims=True)
            return res

        def carried(hprev):
            st = dict(acc=misc_ref[AC, :], l=misc_ref[LC, :])
            out = {}
            for i, (t, x) in enumerate(P.carry):
                p = pc_ref[i]
                if i == NCARRY - 1:
                    p = jnp.exp2(p)
                    for j in range(CK // 16 - 1, -1, -1):
                        st["l"] = st["l"] + (p[j * 16:j * 16 + 8] + p[j * 16 + 8:j * 16 + 16])
                out[x] = (st, hprev, t[0], t[1], p)
            return out

        def head(h, qb_ref, kb_ref, kr_ref, hn, qbn_ref, kbn_ref, krn_ref):
            cpend = carried(jnp.maximum(h - 1, 0))
            fmask = zi_ref[0:8, :] != 0
            fmask4 = jnp.concatenate([fmask] * 4, axis=1)
            st, sv, pg, qhn, ptile, uidx = {}, {}, {}, {}, {}, {}

            ctiles = {P.carry[-1][0]}

            def finish(u, blks, sx):
                xs = [sx[i * 8:(i + 1) * 8] for i in range(len(blks))] if len(blks) > 1 else [sx]
                live = [i for i, (c, b) in enumerate(blks) if (u, c) not in ctiles]
                for i, (c, b) in enumerate(blks):
                    pg[u, c, b] = jnp.exp2(xs[i]) if i in live else xs[i]
                if live:
                    ps = [pg[(u,) + blks[i]] for i in live]
                    t = ps[0] + ps[1] if len(ps) == 2 else ps[0]
                    st[u]["l"] = t if st[u]["l"] is None else st[u]["l"] + t

            def run_segs(key, src):
                for (u2, kb, d0) in P.segpos.get(key, []):
                    if d0 == 0:
                        uidx[u2, kb] = u2 + zs_ref[kb]
                    qb = qb_ref[uidx[u2, kb], d0 * 8:(d0 + SEG) * 8, :]
                    kk = kb_ref[kb, d0 * 8:(d0 + SEG) * 8, :]
                    if src is not None:
                        kk = jnp.concatenate([lax.select(fmask, src, kk[0:8]), kk[8:]], axis=0)
                    pr = jnp.concatenate([kk] * 4, axis=1) * qb
                    for d in range(SEG):
                        t = pr[d * 8:(d + 1) * 8]
                        sv[u2, kb] = sv[u2, kb] + t if (u2, kb) in sv else t

            kro = roll_ko(hn)
            make_kr(krn_ref, hn)
            run_segs(-1, None)
            for (x0, x1) in P.pieces:
                u = P.stream[x0][0]
                if u not in st:
                    st[u] = dict(w=q_weights(kr_ref, u), l=None, acc=misc_ref[ZR, :])
                i0 = x0 - u * P.ng
                kk_ = pltpu.bitcast(kr_ref[i0 * 8:(i0 + x1 - x0) * 8, :], bf16)
                s = jnp.dot(kk_, st[u]["w"], preferred_element_type=f32)
                for x in range(x0, x1):
                    _, blk0, blk1 = P.stream[x]
                    r = (x - x0) * 16
                    for half in range(2):
                        if 2 * x + half in P.segpos:
                            run_segs(2 * x + half, s[r + 8 * half:r + 8 * half + 8, 0:128])
                    finish(u, (blk0, blk1), s[r:r + 16])
                    for (u3, d3) in P.qbpos.get(x, []):
                        if u3 not in qhn:
                            q8 = q_rows(hn, u3)
                            make_wq(krn_ref, q8, u3)
                            qhn[u3] = pltpu.bitcast(q8, bf16).astype(f32)
                        val = jnp.broadcast_to(qhn[u3][d3:d3 + 1, :], (8, TQ))
                        qbn_ref[u3, d3 * 8:(d3 + 1) * 8, :] = lax.select(fmask4, s[r:r + 8], val)
                    if x == KBX:
                        make_kb(kbn_ref, kro)
                    for c in sorted({blk0[0], blk1[0]}):
                        if x == P.last[u, c]:
                            bs = list(range(NV[c]))
                            while bs:
                                take, bs = bs[:2], bs[2:]
                                vals = [sv.pop((u, KB0[c] + b)) for b in take]
                                finish(u, [(c, b) for b in take],
                                       jnp.concatenate(vals, axis=0) if len(vals) > 1 else vals[0])
                            ptile[u, c] = jnp.concatenate(
                                [pg.pop((u, c, b)) for b in range(16)], axis=0)
                if x1 - 1 in cpend:
                    res = do_pv(*cpend.pop(x1 - 1))
                for t in P.pv_after.get(x1 - 1, []):
                    res = do_pv(st[t[0]], h, t[0], t[1], ptile.pop(t))
                for half in range(2):
                    if ('pv', x1 - 1, half) in P.segpos:
                        run_segs(('pv', x1 - 1, half), res[8 * half:8 * half + 8, 0:128])
            misc_ref[AC, :] = st[NQ - 1]["acc"]
            misc_ref[LC, :] = st[NQ - 1]["l"]
            for i, (t, _) in enumerate(P.carry):
                pc_ref[i] = ptile.pop(t)

        def body(i, carry):
            @pl.when(zs_ref[0] == 0)
            def _():
                head(2 * i, qba_ref, kba_ref, kra_ref, 2 * i + 1, qbb_ref, kbb_ref, krb_ref)

            head(2 * i + 1, qbb_ref, kbb_ref, krb_ref, jnp.minimum(2 * i + 2, H - 1),
                 qba_ref, kba_ref, kra_ref)
            return carry

        lax.fori_loop(0, H // 2, body, 0)
        for item in carried(H - 1).values():
            do_pv(*item)
        ob_ref[...] = pltpu.bitcast(o_block(0, 0), u32)

        lall = l_ref[...].reshape(NQ * H, TQ)
        bad_l = jnp.where(jnp.logical_and(lall >= L_LO, lall <= L_HI), 0.0, 1.0)
        bad_v = jnp.where(misc_ref[VM, :] <= V_HI, 0.0, 1.0)
        bad = jnp.maximum(jnp.max(bad_l.reshape(NQ * H // 8, 8, TQ), axis=0), bad_v)

        @pl.when(jnp.max(bad) > 0.0)
        def _exact():
            rowgrp = lax.broadcasted_iota(i32, (64, TQ), 0) // (DH // 2)

            def fb(t, carry):
                u = t // H
                h = t % H
                q = qt_ref[u * 4 + h // 8]
                w = pltpu.bitcast(jnp.where(rowgrp == h % 8, q, jnp.zeros_like(q)), bf16)

                def scores(cb, m):
                    kk = pltpu.bitcast(
                        k_ref[h // 8, pl.ds(pl.multiple_of(cb * 256, 256), 256), :], bf16)
                    s = jnp.dot(kk, w, preferred_element_type=f32)
                    s_ref[pl.ds(pl.multiple_of(cb * 512, 512), 512), :] = s
                    return jnp.maximum(m, jnp.max(s.reshape(64, 8, TQ), axis=0))

                m = lax.fori_loop(0, S // 512, scores, jnp.full((8, TQ), -jnp.inf, f32))
                m = jnp.max(m, axis=0, keepdims=True)

                def pv(cb, la):
                    l, acc = la
                    off = pl.multiple_of(cb * 512, 512)
                    p = jnp.exp2(s_ref[pl.ds(off, 512), :] - m)
                    l = l + jnp.sum(p.reshape(64, 8, TQ), axis=0)
                    vv = pltpu.bitcast(
                        vt_ref[pl.ds(pl.multiple_of(h * 8, 8), 8), pl.ds(off, 512)], bf16)
                    acc = acc + jnp.dot(vv, p.astype(bf16), preferred_element_type=f32)
                    return l, acc

                l, acc = lax.fori_loop(
                    0, S // 512, pv, (jnp.zeros((8, TQ), f32), jnp.zeros((DH, TQ), f32)))
                ot_ref[u, pl.ds(pl.multiple_of(h * DH, DH), DH), :] = acc
                l_ref[u, pl.ds(h, 1), :] = jnp.sum(l, axis=0, keepdims=True)
                return carry

            lax.fori_loop(0, NQ * H, fb, 0)
            ob_ref[...] = pltpu.bitcast(o_block(0, 0), u32)

        for cp in late_copies():
            cp.wait()

    b1 = bias_ref[0:F].astype(f32)[None, :]
    b2 = bias_ref[2048:2048 + D].astype(f32)[None, :]

    def out_copy(j):
        return pltpu.make_async_copy(o_ref.at[j], o_hbm.at[pl.ds(aligned(j * TS, TS), TS), :],
                                     osem.at[j])

    hs, hns = [], []
    for i in range(NSUB):
        r0 = pl.multiple_of(step * TM + i * TS, TS)
        o = pltpu.bitcast(ob_ref[...], bf16) if i == 0 else o_block(step, i)
        attn = jnp.dot(o, wo_ref[...], preferred_element_type=f32)
        h = x_ref[pl.ds(r0, TS), :].astype(f32) + attn
        hs.append(h)
        hns.append(_layernorm(h).astype(bf16))
    for i in range(NSUB):
        a = jnp.dot(hns[i], w1_ref[...], preferred_element_type=f32) + b1
        a = jax.nn.gelu(a, approximate=True).astype(bf16)
        y = jnp.dot(a, w2_ref[...], preferred_element_type=f32) + b2
        o_ref[step * NSUB + i] = (hs[i] + y).astype(o_ref.dtype)
        out_copy(step * NSUB + i).start()
    ob_ref[...] = pltpu.bitcast(o_block(jnp.minimum(step + 1, NB - 1), 0), u32)

    @pl.when(step == NB - 1)
    def _():
        for j in range(NB * NSUB):
            out_copy(j).wait()


@jax.jit
def pallas_sequential_preLN__softmax_full_mha__dense_activation_gelu__prompt_kernel(
    A_x: jax.Array,
    A_wqkv: jax.Array,
    A_wo: jax.Array,
    B_x: jax.Array,
    B_w1: jax.Array,
    B_b1: jax.Array,
    B_w2: jax.Array,
    B_b2: jax.Array,
):
    del B_x
    x = A_x.reshape(S, D)
    hbm = pl.BlockSpec(memory_space=pl.ANY)
    tables = [
        pltpu.VMEM((NQ, DH * 8, TQ), f32),
        pltpu.VMEM((RPAD // 8, DH * 8, 128), f32),
        pltpu.VMEM((1024, 128), u32),
    ]

    out = pl.pallas_call(
        _kernel,
        grid=(NB,),
        in_specs=[hbm] * 7,
        out_specs=hbm,
        out_shape=jax.ShapeDtypeStruct((S, D), A_x.dtype),
        scratch_shapes=[
            pltpu.VMEM((S, D), bf16),
            pltpu.VMEM((D, D), bf16),
            pltpu.VMEM((D, D), bf16),
            pltpu.VMEM((D, D), bf16),
            pltpu.VMEM((D, D), bf16),
            pltpu.VMEM((D, F), bf16),
            pltpu.VMEM((F, D), bf16),
            pltpu.SemaphoreType.DMA((NX + 8,)),
            pltpu.VMEM((S // 2, D), u32),
            pltpu.VMEM((4, S // 2, 128), u32),
            pltpu.VMEM((4, S // 2, 128), u32),
            pltpu.VMEM((NQ * 4, 64, TQ), u32),
            pltpu.VMEM((D // 2, S), u32),
            pltpu.VMEM((4, RPAD, 128), f32),
        ] + tables + tables + [
            pltpu.VMEM((NCARRY, CK, TQ), f32),
            pltpu.VMEM((64, TQ), f32),
            pltpu.VMEM((128, 128), i32),
            pltpu.SMEM((NKB,), i32),
            pltpu.VMEM((NQ, D, TQ), f32),
            pltpu.VMEM((NQ, H, TQ), f32),
            pltpu.VMEM((TS // 2, D), u32),
            pltpu.VMEM((S, TQ), f32),
            pltpu.VMEM((32768,), bf16),
            pltpu.VMEM((S // TS, TS, D), bf16),
            pltpu.SemaphoreType.DMA((S // TS,)),
        ],
        compiler_params=pltpu.CompilerParams(
            dimension_semantics=("arbitrary",),
            vmem_limit_bytes=100 * 1024 * 1024,
        ),
    )(x, A_wqkv, A_wo, B_w1, B_w2, B_b1, B_b2)
    return out.reshape(1, S, D)
```

```python
import jax
import jax.numpy as jnp
from jax import lax
import jax.experimental.pallas as pl
import jax.experimental.pallas.tpu as pltpu

S = 2048
D = 512
H = 32
DH = 16
F = 1792
TQ = 512
NQ = S // TQ
CK = 128
NC = S // CK
TM = 512
NB = S // TM
NSUB = 2
TS = TM // NSUB
XCH = [(0, 256), (256, 256), (512, 512), (1024, 512), (1536, 512)]
NX = len(XCH)
EPS = 1e-5
QSCALE = (DH ** -0.5) * 1.4426950408889634

NV = [2 + c % 2 for c in range(NC)]
KB0 = [sum(NV[:c]) for c in range(NC + 1)]
MB0 = [16 * c - KB0[c] for c in range(NC + 1)]
NKB = KB0[NC]
RV = NKB * 8
RPAD = 384
SEG = 4
SHIFT = 2
LAGG = 8
KBX = 8
L_LO = 2.0 ** -10
L_HI = 2.0 ** 64
V_HI = 2.0 ** 60

f32 = jnp.float32
bf16 = jnp.bfloat16
i32 = jnp.int32
u32 = jnp.uint32


def _layernorm(x):
    m = jnp.mean(x, axis=-1, keepdims=True)
    xc = x - m
    v = jnp.mean(xc * xc, axis=-1, keepdims=True)
    return xc * lax.rsqrt(v + EPS)


class _Plan:
    def __init__(self):
        blocks = [(c, b) for c in range(NC) for b in range(15, NV[c] - 1, -1)]
        assert len(blocks) % 2 == 0
        self.ng = len(blocks) // 2
        self.stream = [(u, blocks[2 * i], blocks[2 * i + 1])
                       for u in range(NQ) for i in range(self.ng)]
        ns = self.ns = len(self.stream)
        self.last, self.lasth = {}, {}
        for x, (u, b0, b1) in enumerate(self.stream):
            for half, (c, b) in enumerate((b0, b1)):
                self.last[u, c] = x
                self.lasth[u, c] = 2 * x + half
        tiles = [(u, c) for u in range(NQ) for c in range(NC)]
        self.pv_after, self.carry = {}, []
        for t in tiles:
            x = self.last[t] + LAGG
            if x <= ns - 1:
                self.pv_after.setdefault(x, []).append(t)
            else:
                self.carry.append((t, x - ns))
        assert all(t[0] == NQ - 1 for t, _ in self.carry)
        cuts = set(self.pv_after) | {x for _, x in self.carry} | {
            x for x in range(ns) if x == ns - 1 or self.stream[x + 1][0] != self.stream[x][0]}
        self.pieces, x0 = [], 0
        for x in range(ns):
            if x in cuts:
                self.pieces.append((x0, x + 1))
                x0 = x + 1
        segs = [(t, kb, d0) for t in tiles
                for kb in range(KB0[t[1]], KB0[t[1] + 1])
                for d0 in range(0, DH, SEG)]
        slots = []
        cx = {x for _, x in self.carry}
        for (x0, x1) in self.pieces:
            slots += list(range(2 * x0, 2 * x1))
            if x1 - 1 in self.pv_after or x1 - 1 in cx:
                slots += [('pv', x1 - 1, 0), ('pv', x1 - 1, 1)]
        sidx = {k: i for i, k in enumerate(slots)}
        self.segpos = {}
        for i, (t, kb, d0) in enumerate(segs):
            pos = min((i * len(slots)) // len(segs) - SHIFT, sidx[self.lasth[t]])
            self.segpos.setdefault(slots[pos] if pos >= 0 else -1, []).append((t[0], kb, d0))
        items = [(u, d) for u in range(NQ) for d in range(DH)]
        self.qbpos = {}
        for i, it in enumerate(items):
            self.qbpos.setdefault((i * (ns - 8)) // len(items), []).append(it)


PLAN = _Plan()
NCARRY = len(PLAN.carry)


def _kernel(x_hbm, wqkv_hbm, wo_hbm, w1_hbm, w2_hbm, b1_hbm, b2_hbm, o_hbm,
            x_ref, wq_ref, wk_ref, wv_ref, wo_ref, w1_ref, w2_ref, sem,
            xn_ref, k_ref, ks_ref, qt_ref, vt_ref, ko_ref,
            qba_ref, kba_ref, kra_ref, qbb_ref, kbb_ref, krb_ref,
            pc_ref, misc_ref, zi_ref, ot_ref, l_ref, ob_ref, s_ref, bias_ref, o_ref, osem):
    step = pl.program_id(0)
    P = PLAN
    AC, ZR, VM, LC = slice(0, 16), slice(16, 32), slice(32, 40), slice(48, 56)
    KL = slice(56, 64)

    def x_copy(i):
        r0, n = XCH[i]
        return pltpu.make_async_copy(x_hbm.at[pl.ds(r0, n), :], x_ref.at[pl.ds(r0, n), :],
                                     sem.at[i])

    def w_copy(i):
        dst = (wq_ref, wk_ref, wv_ref)[i]
        return pltpu.make_async_copy(wqkv_hbm.at[:, pl.ds(i * D, D)], dst, sem.at[NX + i])

    def late_copies():
        return (pltpu.make_async_copy(wo_hbm, wo_ref, sem.at[NX + 3]),
                pltpu.make_async_copy(w1_hbm, w1_ref, sem.at[NX + 4]),
                pltpu.make_async_copy(w2_hbm, w2_ref, sem.at[NX + 5]),
                pltpu.make_async_copy(b1_hbm, bias_ref.at[pl.ds(0, F)], sem.at[NX + 6]),
                pltpu.make_async_copy(b2_hbm, bias_ref.at[pl.ds(2048, D)], sem.at[NX + 7]))

    def aligned(i, m):
        return i if isinstance(i, int) else pl.multiple_of(i, m)

    def head_shift(h):
        return (128 - (h % 8) * DH) % 128

    def q_rows(h, u):
        return qt_ref[u * 4 + h // 8, pl.ds(aligned((h % 8) * 8, 8), 8), :]

    def q_weights(kr_ref, u):
        r0 = (P.ng + 4 * u) * 8
        q8 = jnp.concatenate([kr_ref[r0 + t * 8:r0 + (t + 1) * 8, :] for t in range(4)], axis=1)
        return jnp.concatenate(
            [pltpu.bitcast(q8, bf16), jnp.zeros((128 - DH, TQ), bf16)], axis=0)

    def make_wq(kr_ref, q8, u):
        r0 = (P.ng + 4 * u) * 8
        for t in range(4):
            kr_ref[r0 + t * 8:r0 + (t + 1) * 8, :] = q8[:, t * 128:(t + 1) * 128]

    def roll_ko(h):
        return pltpu.roll(ko_ref[h // 8, 0:RV, :], head_shift(h), 1)

    def make_kb(kb_ref, kro):
        for d in range(DH):
            kb_ref[0:NKB, d * 8:(d + 1) * 8, :] = jnp.broadcast_to(
                kro[:, d:d + 1], (RV, 128)).reshape(NKB, 8, 128)

    def make_kr(kr_ref, h):
        kr_ref[0:P.ng * 8, :] = pltpu.roll(ks_ref[h // 8, 0:P.ng * 8, :], head_shift(h), 1)

    def o_block(u, i):
        linv = 1.0 / l_ref[u, :, i * TS:(i + 1) * TS]
        o = jnp.concatenate(
            [ot_ref[u, h * DH:(h + 1) * DH, i * TS:(i + 1) * TS] * linv[h:h + 1, :]
             for h in range(H)], axis=0)
        return o.T.astype(bf16)

    @pl.when(step == 0)
    def _attention():
        x_copy(0).start()
        w_copy(1).start()
        for i in range(1, NX):
            x_copy(i).start()
        w_copy(0).start()
        w_copy(2).start()

        misc_ref[0:32, :] = jnp.zeros((32, TQ), f32)
        misc_ref[LC, :] = jnp.ones((8, TQ), f32)
        zi_ref[0:8, :] = jnp.zeros((8, 128), i32)
        pc_ref[...] = jnp.zeros_like(pc_ref)

        def ln_chunk(r0, n, pace=None):
            x = x_ref[r0:r0 + n, :].astype(f32)
            if pace is not None:
                fm = zi_ref[0:8, :] != 0
                m, nj = pace.shape[0] // 8, n // 8
                parts = []
                for j in range(nj):
                    pr, pc = (j * 3 * m) // nj % m, (j * 3) // nj
                    parts.append(jnp.where(fm, pace[pr * 8:pr * 8 + 8, pc * 128:pc * 128 + 128],
                                           x[j * 8:(j + 1) * 8, 0:128]))
                x0 = jnp.concatenate(parts, axis=0)
                x = jnp.concatenate([x0, x[:, 128:]], axis=1)
            xn_ref[r0 // 2:(r0 + n) // 2, :] = pltpu.bitcast(_layernorm(x).astype(bf16), u32)

        def k_chunk(r0, n):
            xn = pltpu.bitcast(xn_ref[r0 // 2:(r0 + n) // 2, :], bf16)
            kf = jnp.dot(xn, wk_ref[...], preferred_element_type=f32)
            kb16 = kf.astype(bf16)
            kpk = pltpu.bitcast(kb16, u32)
            c0, c1 = r0 // CK, (r0 + n) // CK
            blks = [kf[(c - c0) * CK + b * 8:(c - c0) * CK + b * 8 + 8]
                    for c in range(c0, c1) for b in range(15, NV[c] - 1, -1)]
            if MB0[c0] % 2:
                blks = [misc_ref[KL, :]] + blks
            if MB0[c1] % 2:
                misc_ref[KL, :] = blks.pop()
            kspk = pltpu.bitcast(jnp.concatenate(blks, axis=0).astype(bf16), u32)
            kof = jnp.concatenate(
                [kf[(c - c0) * CK:(c - c0) * CK + 8 * NV[c]] for c in range(c0, c1)], axis=0)
            kof = kof.astype(bf16).astype(f32)
            for g in range(4):
                k_ref[g, r0 // 2:(r0 + n) // 2, :] = kpk[:, g * 128:(g + 1) * 128]
                ks_ref[g, MB0[c0] // 2 * 8:MB0[c1] // 2 * 8, :] = kspk[:, g * 128:(g + 1) * 128]
                ko_ref[g, KB0[c0] * 8:KB0[c1] * 8, :] = kof[:, g * 128:(g + 1) * 128]
            return kf

        x_copy(0).wait()
        ln_chunk(0, 256)
        w_copy(1).wait()
        x_copy(1).wait()
        ln_chunk(256, 256, k_chunk(0, 256))
        x_copy(2).wait()
        ln_chunk(512, 512, k_chunk(256, 256))
        x_copy(3).wait()
        kf = k_chunk(512, 512)
        ln_chunk(1024, 256)
        ln_chunk(1280, 256, kf)
        k_chunk(1024, 256)
        x_copy(4).wait()
        w_copy(0).wait()
        w_copy(2).wait()
        for cp in late_copies():
            cp.start()
        k_chunk(1280, 256)
        ln_chunk(1536, 512)
        k_chunk(1536, 512)
        wqv_t = jnp.concatenate(
            [wq_ref[...].astype(f32).T.astype(bf16), wv_ref[...].astype(f32).T.astype(bf16)],
            axis=0)
        nt = (((1,), (1,)), ((), ()))
        make_kb(kba_ref, roll_ko(0))
        make_kr(kra_ref, 0)
        for b in range(NQ):
            xn = pltpu.bitcast(xn_ref[b * TQ // 2:(b + 1) * TQ // 2, :], bf16)
            qv = lax.dot_general(wqv_t, xn, nt, preferred_element_type=f32)
            qt = pltpu.bitcast((qv[0:D] * QSCALE).astype(bf16), u32)
            for g in range(4):
                qt_ref[b * 4 + g] = qt[g * 64:(g + 1) * 64, :]
            vt_ref[:, b * TQ:(b + 1) * TQ] = pltpu.bitcast(qv[D:2 * D].astype(bf16), u32)
            va = jnp.max(jnp.abs(qv[D:2 * D]).reshape(D // 8, 8, TQ), axis=0)
            vmax = va if b == 0 else jnp.maximum(vmax, va)
            make_wq(kra_ref, q_rows(0, b), b)
            qh = pltpu.bitcast(q_rows(0, b), bf16).astype(f32)
            for d in range(DH):
                qba_ref[b, d * 8:(d + 1) * 8, :] = jnp.broadcast_to(qh[d:d + 1, :], (8, TQ))

        misc_ref[VM, :] = vmax

        def do_pv(st, h, u, c, p):
            vv = pltpu.bitcast(vt_ref[pl.ds(aligned(h * 8, 8), 8), c * CK:(c + 1) * CK], bf16)
            st["acc"] = st["acc"] + lax.dot_general(
                vv, p, (((1,), (0,)), ((), ())), precision=lax.Precision.DEFAULT,
                preferred_element_type=f32)
            res = st["acc"]
            if c == NC - 1:
                ot_ref[u, pl.ds(aligned(h * DH, DH), DH), :] = st["acc"]
                l_ref[u, pl.ds(h, 1), :] = jnp.sum(st["l"], axis=0, keepdims=True)
            return res

        def carried(hprev):
            st = dict(acc=misc_ref[AC, :], l=misc_ref[LC, :])
            out = {}
            for i, (t, x) in enumerate(P.carry):
                p = pc_ref[i]
                if i == NCARRY - 1:
                    p = jnp.exp2(p)
                    for j in range(CK // 16 - 1, -1, -1):
                        st["l"] = st["l"] + (p[j * 16:j * 16 + 8] + p[j * 16 + 8:j * 16 + 16])
                out[x] = (st, hprev, t[0], t[1], p)
            return out

        def head(h, qb_ref, kb_ref, kr_ref, hn, qbn_ref, kbn_ref, krn_ref):
            cpend = carried(jnp.maximum(h - 1, 0))
            fmask = zi_ref[0:8, :] != 0
            fmask4 = jnp.concatenate([fmask] * 4, axis=1)
            st, sv, pg, qhn, ptile, uidx = {}, {}, {}, {}, {}, {}

            ctiles = {P.carry[-1][0]}

            def finish(u, blks, sx):
                xs = [sx[i * 8:(i + 1) * 8] for i in range(len(blks))] if len(blks) > 1 else [sx]
                live = [i for i, (c, b) in enumerate(blks) if (u, c) not in ctiles]
                for i, (c, b) in enumerate(blks):
                    pg[u, c, b] = jnp.exp2(xs[i]) if i in live else xs[i]
                if live:
                    ps = [pg[(u,) + blks[i]] for i in live]
                    t = ps[0] + ps[1] if len(ps) == 2 else ps[0]
                    st[u]["l"] = t if st[u]["l"] is None else st[u]["l"] + t

            def run_segs(key, src):
                for (u2, kb, d0) in P.segpos.get(key, []):
                    if d0 == 0:
                        uidx[u2, kb] = u2 + lax.shift_right_logical(h + kb, 12)
                    qb = qb_ref[uidx[u2, kb], d0 * 8:(d0 + SEG) * 8, :]
                    kk = kb_ref[kb, d0 * 8:(d0 + SEG) * 8, :]
                    if src is not None:
                        kk = jnp.concatenate([lax.select(fmask, src, kk[0:8]), kk[8:]], axis=0)
                    pr = jnp.concatenate([kk] * 4, axis=1) * qb
                    for d in range(SEG):
                        t = pr[d * 8:(d + 1) * 8]
                        sv[u2, kb] = sv[u2, kb] + t if (u2, kb) in sv else t

            kro = roll_ko(hn)
            make_kr(krn_ref, hn)
            run_segs(-1, None)
            for (x0, x1) in P.pieces:
                u = P.stream[x0][0]
                if u not in st:
                    st[u] = dict(w=q_weights(kr_ref, u), l=None, acc=misc_ref[ZR, :])
                i0 = x0 - u * P.ng
                kk_ = pltpu.bitcast(kr_ref[i0 * 8:(i0 + x1 - x0) * 8, :], bf16)
                s = jnp.dot(kk_, st[u]["w"], preferred_element_type=f32)
                for x in range(x0, x1):
                    _, blk0, blk1 = P.stream[x]
                    r = (x - x0) * 16
                    for half in range(2):
                        if 2 * x + half in P.segpos:
                            run_segs(2 * x + half, s[r + 8 * half:r + 8 * half + 8, 0:128])
                    finish(u, (blk0, blk1), s[r:r + 16])
                    for (u3, d3) in P.qbpos.get(x, []):
                        if u3 not in qhn:
                            q8 = q_rows(hn, u3)
                            make_wq(krn_ref, q8, u3)
                            qhn[u3] = pltpu.bitcast(q8, bf16).astype(f32)
                        val = jnp.broadcast_to(qhn[u3][d3:d3 + 1, :], (8, TQ))
                        qbn_ref[u3, d3 * 8:(d3 + 1) * 8, :] = lax.select(fmask4, s[r:r + 8], val)
                    if x == KBX:
                        make_kb(kbn_ref, kro)
                    for c in sorted({blk0[0], blk1[0]}):
                        if x == P.last[u, c]:
                            bs = list(range(NV[c]))
                            while bs:
                                take, bs = bs[:2], bs[2:]
                                vals = [sv.pop((u, KB0[c] + b)) for b in take]
                                finish(u, [(c, b) for b in take],
                                       jnp.concatenate(vals, axis=0) if len(vals) > 1 else vals[0])
                            ptile[u, c] = jnp.concatenate(
                                [pg.pop((u, c, b)) for b in range(16)], axis=0)
                if x1 - 1 in cpend:
                    res = do_pv(*cpend.pop(x1 - 1))
                for t in P.pv_after.get(x1 - 1, []):
                    res = do_pv(st[t[0]], h, t[0], t[1], ptile.pop(t))
                for half in range(2):
                    if ('pv', x1 - 1, half) in P.segpos:
                        run_segs(('pv', x1 - 1, half), res[8 * half:8 * half + 8, 0:128])
            misc_ref[AC, :] = st[NQ - 1]["acc"]
            misc_ref[LC, :] = st[NQ - 1]["l"]
            for i, (t, _) in enumerate(P.carry):
                pc_ref[i] = ptile.pop(t)

        def body(i, carry):
            @pl.when(i < H)
            def _():
                head(2 * i, qba_ref, kba_ref, kra_ref, 2 * i + 1, qbb_ref, kbb_ref, krb_ref)

            head(2 * i + 1, qbb_ref, kbb_ref, krb_ref, jnp.minimum(2 * i + 2, H - 1),
                 qba_ref, kba_ref, kra_ref)
            return carry

        lax.fori_loop(0, H // 2, body, 0)
        for item in carried(H - 1).values():
            do_pv(*item)
        ob_ref[...] = pltpu.bitcast(o_block(0, 0), u32)

        lall = l_ref[...].reshape(NQ * H, TQ)
        bad_l = jnp.where(jnp.logical_and(lall >= L_LO, lall <= L_HI), 0.0, 1.0)
        bad_v = jnp.where(misc_ref[VM, :] <= V_HI, 0.0, 1.0)
        bad = jnp.maximum(jnp.max(bad_l.reshape(NQ * H // 8, 8, TQ), axis=0), bad_v)

        @pl.when(jnp.max(bad) > 0.0)
        def _exact():
            rowgrp = lax.broadcasted_iota(i32, (64, TQ), 0) // (DH // 2)

            def fb(t, carry):
                u = t // H
                h = t % H
                q = qt_ref[u * 4 + h // 8]
                w = pltpu.bitcast(jnp.where(rowgrp == h % 8, q, jnp.zeros_like(q)), bf16)

                def scores(cb, m):
                    kk = pltpu.bitcast(
                        k_ref[h // 8, pl.ds(pl.multiple_of(cb * 256, 256), 256), :], bf16)
                    s = jnp.dot(kk, w, preferred_element_type=f32)
                    s_ref[pl.ds(pl.multiple_of(cb * 512, 512), 512), :] = s
                    return jnp.maximum(m, jnp.max(s.reshape(64, 8, TQ), axis=0))

                m = lax.fori_loop(0, S // 512, scores, jnp.full((8, TQ), -jnp.inf, f32))
                m = jnp.max(m, axis=0, keepdims=True)

                def pv(cb, la):
                    l, acc = la
                    off = pl.multiple_of(cb * 512, 512)
                    p = jnp.exp2(s_ref[pl.ds(off, 512), :] - m)
                    l = l + jnp.sum(p.reshape(64, 8, TQ), axis=0)
                    vv = pltpu.bitcast(
                        vt_ref[pl.ds(pl.multiple_of(h * 8, 8), 8), pl.ds(off, 512)], bf16)
                    acc = acc + jnp.dot(vv, p.astype(bf16), preferred_element_type=f32)
                    return l, acc

                l, acc = lax.fori_loop(
                    0, S // 512, pv, (jnp.zeros((8, TQ), f32), jnp.zeros((DH, TQ), f32)))
                ot_ref[u, pl.ds(pl.multiple_of(h * DH, DH), DH), :] = acc
                l_ref[u, pl.ds(h, 1), :] = jnp.sum(l, axis=0, keepdims=True)
                return carry

            lax.fori_loop(0, NQ * H, fb, 0)
            ob_ref[...] = pltpu.bitcast(o_block(0, 0), u32)

        for cp in late_copies():
            cp.wait()

    b1 = bias_ref[0:F].astype(f32)[None, :]
    b2 = bias_ref[2048:2048 + D].astype(f32)[None, :]

    def out_copy(j):
        return pltpu.make_async_copy(o_ref.at[j], o_hbm.at[pl.ds(aligned(j * TS, TS), TS), :],
                                     osem.at[j])

    hs, hns = [], []
    for i in range(NSUB):
        r0 = pl.multiple_of(step * TM + i * TS, TS)
        o = pltpu.bitcast(ob_ref[...], bf16) if i == 0 else o_block(step, i)
        attn = jnp.dot(o, wo_ref[...], preferred_element_type=f32)
        h = x_ref[pl.ds(r0, TS), :].astype(f32) + attn
        hs.append(h)
        hns.append(_layernorm(h).astype(bf16))
    for i in range(NSUB):
        a = jnp.dot(hns[i], w1_ref[...], preferred_element_type=f32) + b1
        a = jax.nn.gelu(a, approximate=True).astype(bf16)
        y = jnp.dot(a, w2_ref[...], preferred_element_type=f32) + b2
        o_ref[step * NSUB + i] = (hs[i] + y).astype(o_ref.dtype)
        out_copy(step * NSUB + i).start()
    ob_ref[...] = pltpu.bitcast(o_block(jnp.minimum(step + 1, NB - 1), 0), u32)

    @pl.when(step == NB - 1)
    def _():
        for j in range(NB * NSUB):
            out_copy(j).wait()


@jax.jit
def pallas_sequential_preLN__softmax_full_mha__dense_activation_gelu__prompt_kernel(
    A_x: jax.Array,
    A_wqkv: jax.Array,
    A_wo: jax.Array,
    B_x: jax.Array,
    B_w1: jax.Array,
    B_b1: jax.Array,
    B_w2: jax.Array,
    B_b2: jax.Array,
):
    del B_x
    x = A_x.reshape(S, D)
    hbm = pl.BlockSpec(memory_space=pl.ANY)
    tables = [
        pltpu.VMEM((NQ, DH * 8, TQ), f32),
        pltpu.VMEM((RPAD // 8, DH * 8, 128), f32),
        pltpu.VMEM((1024, 128), u32),
    ]

    out = pl.pallas_call(
        _kernel,
        grid=(NB,),
        in_specs=[hbm] * 7,
        out_specs=hbm,
        out_shape=jax.ShapeDtypeStruct((S, D), A_x.dtype),
        scratch_shapes=[
            pltpu.VMEM((S, D), bf16),
            pltpu.VMEM((D, D), bf16),
            pltpu.VMEM((D, D), bf16),
            pltpu.VMEM((D, D), bf16),
            pltpu.VMEM((D, D), bf16),
            pltpu.VMEM((D, F), bf16),
            pltpu.VMEM((F, D), bf16),
            pltpu.SemaphoreType.DMA((NX + 8,)),
            pltpu.VMEM((S // 2, D), u32),
            pltpu.VMEM((4, S // 2, 128), u32),
            pltpu.VMEM((4, S // 2, 128), u32),
            pltpu.VMEM((NQ * 4, 64, TQ), u32),
            pltpu.VMEM((D // 2, S), u32),
            pltpu.VMEM((4, RPAD, 128), f32),
        ] + tables + tables + [
            pltpu.VMEM((NCARRY, CK, TQ), f32),
            pltpu.VMEM((64, TQ), f32),
            pltpu.VMEM((128, 128), i32),
            pltpu.VMEM((NQ, D, TQ), f32),
            pltpu.VMEM((NQ, H, TQ), f32),
            pltpu.VMEM((TS // 2, D), u32),
            pltpu.VMEM((S, TQ), f32),
            pltpu.VMEM((32768,), bf16),
            pltpu.VMEM((S // TS, TS, D), bf16),
            pltpu.SemaphoreType.DMA((S // TS,)),
        ],
        compiler_params=pltpu.CompilerParams(
            dimension_semantics=("arbitrary",),
            vmem_limit_bytes=100 * 1024 * 1024,
        ),
    )(x, A_wqkv, A_wo, B_w1, B_w2, B_b1, B_b2)
    return out.reshape(1, S, D)
```
